```python
import os as _os
_os.environ.setdefault("JAX_PLATFORMS", "cpu")
import jax
import jax.numpy as jnp

def _softmax(x, axis=-1):
    return jax.nn.softmax(x, axis=axis)
def _gelu(x):
    return jax.nn.gelu(x, approximate=True)
def _silu(x):
    return jax.nn.silu(x)
def _sigmoid(x):
    return jax.nn.sigmoid(x)
def _layernorm(x, axis=-1, eps=1e-5):
    m = jnp.mean(x, axis=axis, keepdims=True)
    v = jnp.var(x, axis=axis, keepdims=True)
    return (x - m) / jnp.sqrt(v + eps)
def _scatter_add(tgt, idx, src, axis=0):
    return tgt.at[idx].add(src)
def _segment_sum(src, seg, n):
    return jax.ops.segment_sum(src, seg, n)
class _Rng:
    def __init__(self, key):
        self._k = key
    def _next(self):
        self._k, sub = jax.random.split(self._k)
        return sub
    def normal(self, shape):
        return jax.random.normal(self._next(), shape, dtype=jnp.bfloat16)
    def randint(self, lo, hi, shape):
        return jax.random.randint(self._next(), shape, lo, hi, dtype=jnp.int32)
    def uniform(self, shape, lo=0.0, hi=1.0):
        return jax.random.uniform(self._next(), shape, jnp.bfloat16, lo, hi)
    def permutation(self, n):
        return jax.random.permutation(self._next(), n)


kernel_name = 'gated_mix__ssm_conv_h3__mha_block__prompt'

def setup_inputs():
    _rng = _Rng(jax.random.key(int.from_bytes(__import__("os").urandom(4), "little")))
    _w = (lambda a: (lambda t: t.astype(jnp.bfloat16) if jnp.issubdtype(t.dtype, jnp.floating) else t)(jnp.asarray(a)))
    def _A_setup():
        B, S, D = 1, 2048, 640
        ks = 4
        return {
            "q": _w((lambda *s: _rng.normal(s) * 0.05)(B, S, D)),
            "k": _w((lambda *s: _rng.normal(s) * 0.4)(B, S, D)),
            "v": _w((lambda *s: _rng.normal(s) * 0.4)(B, S, D)),
            "shift_k": _w((lambda *s: _rng.normal(s) * 0.4)(D, ks) * 0.5),
            "ssm_k": _w((lambda *s: _rng.normal(s) * 0.4)(D, S) * (1.0 / S ** 0.5)),
            "ssm_D": _w((lambda *s: _rng.normal(s) * 0.4)(D)),
        }
    _A_in = _A_setup()

    def _B_setup():
        B, S, D, H = 1, 2048, 640, 32
        return {
            "x": _w((lambda *s: _rng.normal(s) * 0.05)(B, S, D)),
            "wqkv": _w((lambda *s: _rng.normal(s) * 0.4)(D, 3 * D)),
            "wo": _w((lambda *s: _rng.normal(s) * 0.05)(D, D)),
        }
    _B_in = _B_setup()

    return {
        "A_q": _A_in["q"],
        "A_k": _A_in["k"],
        "A_v": _A_in["v"],
        "A_shift_k": _A_in["shift_k"],
        "A_ssm_k": _A_in["ssm_k"],
        "A_ssm_D": _A_in["ssm_D"],
        "B_x": _B_in["x"],
        "B_wqkv": _B_in["wqkv"],
        "B_wo": _B_in["wo"],
        "gate_w": _w((lambda *s: _rng.normal(s) * 0.05)(640) * 16.0),
    }

def reference(A_q, A_k, A_v, A_shift_k, A_ssm_k, A_ssm_D, B_x, B_wqkv, B_wo, gate_w):
    def _A_ref(q, k, v, shift_k, ssm_k, ssm_D):
        B, S, D = q.shape
        ks = shift_k.shape[-1]
        k_pad = jnp.pad(k, ((0, 0), (ks - 1, 0), (0, 0)))
        k_shift = jnp.zeros_like(k)
        for t in range(ks):
            k_shift = k_shift + k_pad[:, t:t + S, :] * shift_k[:, ks - 1 - t][None, None, :]
        kv = k_shift * v
        L = 2 * S
        kv_pad = jnp.pad(kv, ((0, 0), (0, S), (0, 0)))
        kf_pad = jnp.pad(ssm_k, ((0, 0), (0, S)))
        kv_f = (lambda x, axes=(-2,-1): jnp.fft.rfft2(x.astype(jnp.float32), axes=axes))(kv_pad[:, None, :, :], axes=(1, 2))
        kf_f = (lambda x, axes=(-2,-1): jnp.fft.rfft2(x.astype(jnp.float32), axes=axes))(kf_pad[:, None, :], axes=(1, 2))
        kf_f = (lambda x, *d: x.transpose(*d))(kf_f, 1, 2, 0)
        y_f = kv_f * kf_f[None, :, :, :]
        y = (lambda x, s, axes=(-2,-1): jnp.fft.irfft2(x, s=s, axes=axes).astype(jnp.bfloat16))(y_f, (1, L), axes=(1, 2))[:, 0, :S, :]
        y = y + kv * ssm_D[None, None, :]
        return q * y

    def _B_ref(x, wqkv, wo):
        B, S, D = x.shape
        H = 32
        Dh = D // H
        qkv = (lambda x, *d: x.transpose(*d))((x @ wqkv).reshape(B, S, 3, H, Dh), 2, 0, 3, 1, 4)
        q, k, v = qkv[0], qkv[1], qkv[2]
        scores = jnp.einsum("bhqd,bhkd->bhqk", q, k) * (Dh ** -0.5)
        p = _softmax(scores, axis=-1)
        o = jnp.einsum("bhqk,bhkd->bhqd", p, v)
        return (lambda x, *d: x.transpose(*d))(o, 0, 2, 1, 3).reshape(B, S, D) @ wo

    x = A_q
    g = _sigmoid((x * gate_w).sum(-1, keepdims=True))
    a = _A_ref(x, A_k, A_v, A_shift_k, A_ssm_k, A_ssm_D)
    b = _B_ref(x, B_wqkv, B_wo)
    return g * a + (1 - g) * b
```

```python
import functools
import math

import numpy as np
import jax
import jax.numpy as jnp
from jax import lax
import jax.experimental.pallas as pl
import jax.experimental.pallas.tpu as pltpu

S = 2048
D = 640
H = 32
DH = 20
NG = 6
TQ = 512
NQ = S // TQ
KC = 128
NC = S // KC
B = 128
NB = S // B
XC = 512
NX = S // XC
BPC = XC // B

F32 = jnp.float32
BF16 = jnp.bfloat16
U32 = jnp.uint32


def _dft_consts():
    r = np.arange(2 * B)
    t, part, i = r // 16, (r // 8) % 2, r % 8
    f = np.where(t < 8, 2 * (8 * t + i), 2 * (8 * (t - 8) + i) + 1)
    theta = np.pi * (2 * f + 1) / (2 * B)
    j = np.arange(B)
    ang = theta[:, None] * j[None, :]
    fwd = np.where(part[:, None] == 0, np.cos(ang), -np.sin(ang))
    inv = fwd.T / B
    return fwd.astype(np.float32), inv.astype(np.float32)


def _bf(x):
    return pltpu.bitcast(x, BF16)


def _u32(x):
    return pltpu.bitcast(x, U32)


def _kernel(x_hbm, k_hbm, v_hbm, ssm_hbm, wqkv_hbm, wo_hbm,
            shift_ref, dvec_ref, gw_ref, fwd_ref, inv_ref,
            out_hbm,
            x_v, k_v, v_v, ssm_v, wqkv_v, wo_v, out_v,
            wk_s, wt_s, qt_s, kk_s, vt_s, s0, s1, m0, m1, ot_s,
            u_s, kf_s, kp_s, y_s, kv_s, kpad_s,
            sem_w, sem_x, sem_o):
    cp_wqkv = pltpu.make_async_copy(wqkv_hbm, wqkv_v, sem_w.at[0])
    cp_wo = pltpu.make_async_copy(wo_hbm, wo_v, sem_w.at[1])

    def chunk_copies(i):
        rows = pl.ds(pl.multiple_of(i * XC, XC), XC)
        return [
            pltpu.make_async_copy(x_hbm.at[0, rows, :], x_v.at[rows, :], sem_x.at[4 * i]),
            pltpu.make_async_copy(ssm_hbm.at[:, rows], ssm_v.at[:, rows], sem_x.at[4 * i + 1]),
            pltpu.make_async_copy(k_hbm.at[0, rows, :], k_v.at[rows, :], sem_x.at[4 * i + 2]),
            pltpu.make_async_copy(v_hbm.at[0, rows, :], v_v.at[rows, :], sem_x.at[4 * i + 3]),
        ]

    cp_wqkv.start()
    for i in range(NX):
        for c in chunk_copies(i):
            c.start()
    cp_wo.start()

    s1[...] = jnp.zeros_like(s1)
    m1[...] = jnp.zeros_like(m1)
    kp_s[0] = jnp.zeros((2 * B, D), F32)
    kf_s[...] = jnp.zeros((2 * B, D), F32)
    kpad_s[0:8, :] = jnp.zeros((8, D), F32)

    cp_wqkv.wait()
    for g in range(NG):
        wk_s[:, g * 128:(g + 1) * 128] = wqkv_v[:, D + 120 * g:D + 120 * g + 128]
    wt_s[0:D, :] = wqkv_v[:, 0:D].astype(F32).T.astype(BF16)
    wt_s[D:2 * D, :] = wqkv_v[:, 2 * D:3 * D].astype(F32).T.astype(BF16)

    qscale = (DH ** -0.5) * math.log2(math.e)

    def prologue(i, carry):
        for c in chunk_copies(i):
            c.wait()
        r0 = pl.multiple_of(i * XC, XC)
        rows = pl.ds(r0, XC)
        x = x_v[rows, :]
        kk = jnp.dot(x, wk_s[...], preferred_element_type=F32).astype(BF16)
        hrows = pl.ds(pl.multiple_of(i * (XC // 2), XC // 2), XC // 2)
        for g in range(NG):
            kk_s[g, hrows, :] = _u32(kk[:, g * 128:(g + 1) * 128])
        qv = lax.dot_general(wt_s[...], x, (((1,), (1,)), ((), ())),
                             preferred_element_type=F32)
        row = lax.broadcasted_iota(jnp.int32, (128, XC), 0)
        ones_tile = jnp.where(lax.broadcasted_iota(jnp.int32, (8, XC), 0) == 0, 1.0, 0.0).astype(F32)
        for h in range(H):
            g, j = h // 6, h % 6
            qg = qv[120 * g:120 * g + 128, :] * qscale
            qm = jnp.where((row >= DH * j) & (row < DH * j + DH), qg, 0.0)
            qt_s[h, :, rows] = _u32(qm.astype(BF16))
            w = (DH * h) // 8 * 8
            vt = jnp.concatenate([qv[D + w:D + w + 24, :], ones_tile], axis=0)
            vt_s[h, :, rows] = _u32(vt.astype(BF16))
        kf32 = k_v[rows, :].astype(F32)
        kpad_s[8:8 + XC, :] = kf32
        sh = shift_ref[...].astype(F32)
        ks = kf32 * sh[0:1, :]
        for l in range(1, 4):
            ks = ks + kpad_s[8 - l:8 - l + XC, :] * sh[l:l + 1, :]
        kpad_s[0:8, :] = kf32[XC - 8:XC, :]
        kv = (ks * v_v[rows, :].astype(F32)).astype(BF16)
        kv_s[rows, :] = kv
        fwd = fwd_ref[...]
        prev = kf_s[...].reshape(16, 2, 8, D)
        for bb in range(BPC):
            b = i * BPC + bb
            u_s[b] = jnp.dot(fwd, kv[bb * B:(bb + 1) * B, :], preferred_element_type=F32)
            kc = lax.dot_general(fwd, ssm_v[:, pl.ds(pl.multiple_of(r0 + bb * B, B), B)],
                                 (((1,), (1,)), ((), ())), preferred_element_type=F32)
            cur = kc.reshape(16, 2, 8, D)
            re = jnp.concatenate([cur[:8, 0] - prev[:8, 1], cur[8:, 0] + prev[8:, 1]], axis=0)
            im = jnp.concatenate([cur[:8, 1] + prev[:8, 0], cur[8:, 1] - prev[8:, 0]], axis=0)
            kp_s[b + 1] = jnp.stack([re, im], axis=1).reshape(2 * B, D)
            prev = cur
        kf_s[...] = prev.reshape(2 * B, D)
        return carry

    lax.fori_loop(0, NX, prologue, 0)

    sb = [s0, s1]
    mb = [m0, m1]

    def s1_chunk(h, g, qi, c, s_ref, m, z):
        s = jnp.dot(_bf(kk_s[g, c * KC // 2:(c + 1) * KC // 2, :]),
                    _bf(qt_s[h, :, qi * TQ:(qi + 1) * TQ]), preferred_element_type=F32)
        s_ref[z, c * KC:(c + 1) * KC, :] = s
        mc = jnp.max(s.reshape(KC // 8, 8, TQ), axis=0)
        return mc if m is None else jnp.maximum(m, mc)

    def s2_chunk(h, c, s_ref, m, acc, z):
        p = jnp.exp2(s_ref[z, c * KC:(c + 1) * KC, :] - m).astype(BF16)
        o = jnp.dot(_bf(vt_s[h, :, c * KC:(c + 1) * KC]), p, preferred_element_type=F32)
        return o if acc is None else acc + o

    def mac_task(ft, par, i, dt):
        fr = pl.ds(pl.multiple_of(ft * 16, 16), 8)
        fi = pl.ds(pl.multiple_of(ft * 16 + 8, 8), 8)
        ln = slice(dt * 128, (dt + 1) * 128)
        yr = None
        yi = None
        for b in range(2 * i + 2):
            kidx = 2 * i + 1 - b + par
            kr = kp_s[kidx, fr, ln]
            ki = kp_s[kidx, fi, ln]
            ur = u_s[b, fr, ln]
            ui = u_s[b, fi, ln]
            tr = kr * ur - ki * ui
            ti = kr * ui + ki * ur
            yr = tr if yr is None else yr + tr
            yi = ti if yi is None else yi + ti
        y = jnp.concatenate([yr, yi], axis=0).astype(BF16)
        y_s[2 * i + par, pl.ds(pl.multiple_of(ft * 8, 8), 8), ln] = _u32(y)

    def fused(h1, g1, q1, h2, q2, z1, z2, tasks):
        sA, mA = sb[q1 % 2], mb[q1 % 2]
        sB, mB = sb[q2 % 2], mb[q2 % 2]
        mcur = mB[...]
        m = None
        acc = None
        for c in range(NC):
            if h1 is not None:
                m = s1_chunk(h1, g1, q1, c, sA, m, z1)
            acc = s2_chunk(h2, c, sB, mcur, acc, z2)
            if c >= 2 and c - 2 < len(tasks):
                tasks[c - 2]()
        if h1 is not None:
            mA[...] = jnp.max(m, axis=0, keepdims=True)
        o = acc[0:24, :] * pl.reciprocal(acc[24:25, :], approx=False)
        r = h2 * DH
        w = pl.multiple_of((r >> 3) << 3, 8)
        off = r & 7
        row = lax.broadcasted_iota(jnp.int32, (24, TQ), 0)
        msk = (row >= off) & (row < off + DH)
        pltpu.store(ot_s.at[pl.ds(w, 24), q2 * TQ:(q2 + 1) * TQ], o, mask=msk)

    def body(h, carry):
        g = (h * 43) >> 8
        z1 = h >> 10
        z2 = h >> 11
        ft = h >> 1
        par = h & 1
        for qi in range(NQ):
            tasks = [functools.partial(mac_task, ft, par, i, dt)
                     for dt in range(5) for i in (qi, 7 - qi)]
            if qi == 0:
                fused(h, g, 0, jnp.maximum(h - 1, 0), NQ - 1, z1, z2, tasks)
            else:
                fused(h, g, qi, h, qi - 1, z1, z2, tasks)
        return carry

    lax.fori_loop(0, H, body, 0)
    fused(None, None, 0, jnp.int32(H - 1), NQ - 1, 0, 0, [])

    cp_wo.wait()

    def out_copy(i):
        rows = pl.ds(pl.multiple_of(i * XC, XC), XC)
        return pltpu.make_async_copy(out_v.at[rows, :], out_hbm.at[0, rows, :], sem_o.at[i])

    def epilogue(i, carry):
        r0 = pl.multiple_of(i * XC, XC)
        rows = pl.ds(r0, XC)
        o = ot_s[:, rows].T.astype(BF16)
        bres = jnp.dot(o, wo_v[...], preferred_element_type=F32)
        inv = inv_ref[...]
        ys = []
        for bb in range(BPC):
            ys.append(jnp.dot(inv, _bf(y_s[i * BPC + bb]), preferred_element_type=F32))
        y = jnp.concatenate(ys, axis=0)
        x = x_v[rows, :].astype(F32)
        y = y + kv_s[rows, :].astype(F32) * dvec_ref[...].astype(F32)
        a = x * y
        logit = jnp.sum(x * gw_ref[...].astype(F32), axis=-1, keepdims=True)
        gate = jax.nn.sigmoid(logit)
        out_v[rows, :] = (bres + gate * (a - bres)).astype(BF16)
        out_copy(i).start()
        return carry

    lax.fori_loop(0, NX, epilogue, 0)
    for i in range(NX):
        out_copy(i).wait()


@jax.jit
def pallas_gated_mix__ssm_conv_h3__mha_block__prompt_kernel(
    A_q, A_k, A_v, A_shift_k, A_ssm_k, A_ssm_D, B_x, B_wqkv, B_wo, gate_w,
):
    del B_x
    fwd, inv = _dft_consts()
    any_spec = pl.BlockSpec(memory_space=pl.ANY)
    vm = pl.BlockSpec(memory_space=pltpu.VMEM)
    scratch = [
        pltpu.VMEM((S, D), BF16),
        pltpu.VMEM((S, D), BF16),
        pltpu.VMEM((S, D), BF16),
        pltpu.VMEM((D, S), BF16),
        pltpu.VMEM((D, 3 * D), BF16),
        pltpu.VMEM((D, D), BF16),
        pltpu.VMEM((S, D), BF16),
        pltpu.VMEM((D, NG * 128), BF16),
        pltpu.VMEM((2 * D, D), BF16),
        pltpu.VMEM((H, 64, S), U32),
        pltpu.VMEM((NG, S // 2, 128), U32),
        pltpu.VMEM((H, 16, S), U32),
        pltpu.VMEM((1, S, TQ), F32),
        pltpu.VMEM((1, S, TQ), F32),
        pltpu.VMEM((1, TQ), F32),
        pltpu.VMEM((1, TQ), F32),
        pltpu.VMEM((D, S), F32),
        pltpu.VMEM((NB, 2 * B, D), F32),
        pltpu.VMEM((2 * B, D), F32),
        pltpu.VMEM((NB + 1, 2 * B, D), F32),
        pltpu.VMEM((NB, B, D), U32),
        pltpu.VMEM((S, D), BF16),
        pltpu.VMEM((XC + 8, D), F32),
        pltpu.SemaphoreType.DMA((2,)),
        pltpu.SemaphoreType.DMA((4 * NX,)),
        pltpu.SemaphoreType.DMA((NX,)),
    ]
    return pl.pallas_call(
        _kernel,
        out_shape=jax.ShapeDtypeStruct((1, S, D), BF16),
        in_specs=[any_spec] * 6 + [vm] * 5,
        out_specs=any_spec,
        scratch_shapes=scratch,
        compiler_params=pltpu.CompilerParams(vmem_limit_bytes=120 * 2 ** 20),
    )(A_q, A_k, A_v, A_ssm_k, B_wqkv, B_wo,
      A_shift_k.T, A_ssm_D.reshape(1, D), gate_w.reshape(1, D),
      jnp.asarray(fwd, BF16), jnp.asarray(inv, BF16))
```

```python
import functools
import math
import os as _os_

import numpy as np
import jax
import jax.numpy as jnp
from jax import lax
import jax.experimental.pallas as pl
import jax.experimental.pallas.tpu as pltpu

S = 2048
D = 640
H = 32
DH = 20
NG = 6
TQ = 512
NQ = S // TQ
NT = TQ // 128
KC = 128
NC = S // KC
B = 128
NB = S // B
XC = 512
NX = S // XC
BPC = XC // B
NVB = int(_os_.environ.get("NVB", "16"))
LAG = int(_os_.environ.get("LAG", "1"))
REV = int(_os_.environ.get("REV", "1"))
SKIP0 = int(_os_.environ.get("SKIP0", "1"))
GRP = int(_os_.environ.get("GRP", "1"))
AHEAD = int(_os_.environ.get("AHEAD", "0"))
KB0 = int(_os_.environ.get("KB0", "2"))
KBS = int(_os_.environ.get("KBS", "3"))
GATE = int(_os_.environ.get("GATE", "1"))
ANCH = int(_os_.environ.get("ANCH", "2"))
KANCH = int(_os_.environ.get("KANCH", "0"))
LINK = int(_os_.environ.get("LINK", "0"))
VLAST = int(_os_.environ.get("VLAST", "0"))
VROW = [int(x) for x in _os_.environ.get("VROW", "2,5,8,11").split(",")]
MROW = int(_os_.environ.get("MROW", "0"))
FORCE = _os_.environ.get("FORCE", "")
VCH = [c for c in range(NC) if (c * NVB) // NC != ((c + 1) * NVB) // NC]

F32 = jnp.float32
BF16 = jnp.bfloat16
U32 = jnp.uint32


def _dft_consts():
    r = np.arange(2 * B)
    t, part, i = r // 16, (r // 8) % 2, r % 8
    f = np.where(t < 8, 2 * (8 * t + i), 2 * (8 * (t - 8) + i) + 1)
    theta = np.pi * (2 * f + 1) / (2 * B)
    j = np.arange(B)
    ang = theta[:, None] * j[None, :]
    fwd = np.where(part[:, None] == 0, np.cos(ang), -np.sin(ang))
    inv = fwd.T / B
    return fwd.astype(np.float32), inv.astype(np.float32)


def _bf(x):
    return pltpu.bitcast(x, BF16)


def _u32(x):
    return pltpu.bitcast(x, U32)


def _kernel(x_hbm, k_hbm, v_hbm, ssm_hbm, wqkv_hbm, wo_hbm,
            shift_ref, dvec_ref, gw_ref, fwd_ref, inv_ref,
            out_hbm,
            x_v, k_v, v_v, ssm_v, wqkv_v, wo_v, out_v,
            wk_s, wt_s, qt_s, kk_s, vt_s, s0, s1, m0, m1, ot_s,
            w_s, kf_s, y_s, kv_s, kpad_s, qf_s, mx_s,
            sem_w, sem_x, sem_o, *kb_s):
    cp_wqkv = pltpu.make_async_copy(wqkv_hbm, wqkv_v, sem_w.at[0])
    cp_wo = pltpu.make_async_copy(wo_hbm, wo_v, sem_w.at[1])

    def chunk_copies(i):
        rows = pl.ds(pl.multiple_of(i * XC, XC), XC)
        return [
            pltpu.make_async_copy(x_hbm.at[0, rows, :], x_v.at[rows, :], sem_x.at[4 * i]),
            pltpu.make_async_copy(ssm_hbm.at[:, rows], ssm_v.at[:, rows], sem_x.at[4 * i + 1]),
            pltpu.make_async_copy(k_hbm.at[0, rows, :], k_v.at[rows, :], sem_x.at[4 * i + 2]),
            pltpu.make_async_copy(v_hbm.at[0, rows, :], v_v.at[rows, :], sem_x.at[4 * i + 3]),
        ]

    cp_wqkv.start()

    s1[...] = jnp.zeros_like(s1)
    m1[...] = jnp.zeros_like(m1)
    w_s[:, :, 0:2] = jnp.zeros((16, 5, 2, 8, 128), F32)
    kf_s[...] = jnp.zeros((2 * B, D), F32)
    kpad_s[0:8, :] = jnp.zeros((8, D), F32)
    mx_s[...] = jnp.zeros_like(mx_s)

    cp_wqkv.wait()
    for c in chunk_copies(0):
        c.start()
    for g in range(NG):
        wk_s[:, g * 128:(g + 1) * 128] = wqkv_v[:, D + 120 * g:D + 120 * g + 128]
    wt_s[0:D, :] = wqkv_v[:, 0:D].astype(F32).T.astype(BF16)
    wt_s[D:2 * D, :] = wqkv_v[:, 2 * D:3 * D].astype(F32).T.astype(BF16)

    qscale = (DH ** -0.5) * math.log2(math.e)

    def absmax8(a):
        a = jnp.abs(a)
        a = jnp.max(a.reshape(a.shape[0] // 8, 8, a.shape[1]), axis=0)
        r = a[:, 0:128]
        for t in range(1, a.shape[1] // 128):
            r = jnp.maximum(r, a[:, t * 128:(t + 1) * 128])
        return r

    def prologue(i, carry):
        for c in chunk_copies(i):
            c.wait()

        @pl.when(i + 1 < NX)
        def _():
            for c in chunk_copies(i + 1):
                c.start()

        r0 = pl.multiple_of(i * XC, XC)
        rows = pl.ds(r0, XC)
        x = x_v[rows, :]
        kf = jnp.dot(x, wk_s[...], preferred_element_type=F32)
        mx_s[1] = jnp.maximum(mx_s[1], absmax8(kf))
        kk = _u32(kf.astype(BF16))
        for cc in range(XC // KC):
            for e in range(8):
                src = cc * 8 + e
                dst = cc * 8 + (7 - e if REV else e)
                drow = pl.ds(pl.multiple_of(i * (XC // 2) + dst * 8, 8), 8)
                for g in range(NG):
                    kk_s[g, drow, :] = kk[src * 8:src * 8 + 8, g * 128:(g + 1) * 128]
        qv = lax.dot_general(wt_s[...], x, (((1,), (1,)), ((), ())),
                             preferred_element_type=F32)
        qs = qv[0:D + 128, :] * qscale
        mx_s[0] = jnp.maximum(mx_s[0], absmax8(qs[0:D, :]))
        mx_s[2] = jnp.maximum(mx_s[2], absmax8(qv[D:2 * D, :]))
        row = lax.broadcasted_iota(jnp.int32, (128, XC), 0)
        row8 = lax.broadcasted_iota(jnp.int32, (8, XC), 0)
        for h in range(H):
            g, j = h // 6, h % 6
            qg = qs[120 * g:120 * g + 128, :]
            qm = jnp.where((row >= DH * j) & (row < DH * j + DH), qg, 0.0)
            qt_s[h, :, rows] = _u32(qm.astype(BF16))
            qf_s[h, 0:DH, rows] = qs[DH * h:DH * h + DH, :]
            w = (DH * h) // 8 * 8
            win = qv[D + w:D + w + 24, :]
            if h % 2 == 0:
                parts = [win[0:16], jnp.where(row8 == 4, 1.0, win[16:24])]
            else:
                parts = [jnp.where(row8 == 0, 1.0, win[0:8]), win[8:24]]
            vt = jnp.concatenate(parts + [jnp.zeros((8, XC), F32)], axis=0)
            vt_s[h, :, rows] = _u32(vt.astype(BF16))
        kf32 = k_v[rows, :].astype(F32)
        kpad_s[8:8 + XC, :] = kf32
        sh = shift_ref[...].astype(F32)
        ks = kf32 * sh[0:1, :]
        for l in range(1, 4):
            ks = ks + kpad_s[8 - l:8 - l + XC, :] * sh[l:l + 1, :]
        kpad_s[0:8, :] = kf32[XC - 8:XC, :]
        kv = (ks * v_v[rows, :].astype(F32)).astype(BF16)
        kv_s[rows, :] = kv
        fwd = fwd_ref[...]
        prev = kf_s[...].reshape(16, 2, 8, D)
        for bb in range(BPC):
            b = i * BPC + bb
            ub = jnp.dot(fwd, kv[bb * B:(bb + 1) * B, :], preferred_element_type=F32)
            ub = ub.reshape(16, 2, 8, D)
            for dt in range(5):
                w_s[:, dt, pl.ds(4 * b + 2, 2)] = ub[:, :, :, dt * 128:(dt + 1) * 128]
            kc = lax.dot_general(fwd, ssm_v[:, pl.ds(pl.multiple_of(r0 + bb * B, B), B)],
                                 (((1,), (1,)), ((), ())), preferred_element_type=F32)
            cur = kc.reshape(16, 2, 8, D)
            re = jnp.concatenate([cur[:8, 0] - prev[:8, 1], cur[8:, 0] + prev[8:, 1]], axis=0)
            im = jnp.concatenate([cur[:8, 1] + prev[:8, 0], cur[8:, 1] - prev[8:, 0]], axis=0)
            kp = jnp.stack([re, im], axis=1)
            for dt in range(5):
                w_s[:, dt, pl.ds(4 * b + 4, 2)] = kp[:, :, :, dt * 128:(dt + 1) * 128]
            prev = cur
        kf_s[...] = prev.reshape(2 * B, D)
        return carry

    lax.fori_loop(0, NX, prologue, 0)
    cp_wo.start()

    def unrev(s):
        if not REV:
            return s
        n = s.shape[0] // 16
        return jnp.concatenate([s[16 * e:16 * e + 16] for e in reversed(range(n))], axis=0)

    def zero_bits(u):
        return lax.shift_right_logical(lax.shift_right_logical(u, U32(31)), U32(1))

    def mac_task(ft, par, i, dt):
        ln = slice(dt * 128, (dt + 1) * 128)
        yr = None
        yi = None
        nb = 2 * i + 1 if (isinstance(par, int) and par == 0) else 2 * i + 2
        for b in range(nb):
            kidx = 4 * (2 * i + 1 - b + par)
            kr = w_s[ft, dt, kidx]
            ki = w_s[ft, dt, kidx + 1]
            ur = w_s[ft, dt, 4 * b + 2]
            ui = w_s[ft, dt, 4 * b + 3]
            tr = kr * ur - ki * ui
            ti = kr * ui + ki * ur
            yr = tr if yr is None else yr + tr
            yi = ti if yi is None else yi + ti
        y = jnp.concatenate([yr, yi], axis=0).astype(BF16)
        yu = _u32(y)
        y_s[2 * i + par, pl.ds(pl.multiple_of(ft * 8, 8), 8), ln] = yu
        return zero_bits(yu)

    def mac_tasks(ft, par, qi):
        return [functools.partial(mac_task, ft, par, i, dt)
                for dt in range(5) for i in (qi, 7 - qi)]

    def finish(acc, ft, par, q2):
        if isinstance(par, int):
            den = acc[20:21, :] if par == 0 else acc[0:1, :]
        else:
            den = jnp.where(par == 0, acc[20:21, :], acc[0:1, :])
        o = acc * pl.reciprocal(den, approx=False)
        w = pl.multiple_of(ft * 40 + par * 16, 8)
        row = lax.broadcasted_iota(jnp.int32, (24, TQ), 0)
        msk = (row >= 4 * par) & (row < 4 * par + DH)
        pltpu.store(ot_s.at[pl.ds(w, 24), q2 * TQ:(q2 + 1) * TQ], o, mask=msk)

    def pv(h, c, p, acc):
        o = jnp.dot(_bf(vt_s[h, :, c * KC:(c + 1) * KC]), p, preferred_element_type=F32)[0:24]
        return o if acc is None else acc + o

    def slow_path():
        sb = [s0, s1]
        mb = [m0, m1]

        def fused(h1, g1, q1, h2, q2, z1, z2, tasks):
            sA, mA = sb[q1 % 2], mb[q1 % 2]
            sB, mB = sb[q2 % 2], mb[q2 % 2]
            mcur = mB[0:1, :]
            m = None
            acc = None
            for c in range(NC):
                if h1 is not None:
                    s = jnp.dot(_bf(kk_s[g1, c * KC // 2:(c + 1) * KC // 2, :]),
                                _bf(qt_s[h1, :, q1 * TQ:(q1 + 1) * TQ]), preferred_element_type=F32)
                    sA[z1, c * KC:(c + 1) * KC, :] = unrev(s)
                    mc = jnp.max(s.reshape(KC // 8, 8, TQ), axis=0)
                    m = mc if m is None else jnp.maximum(m, mc)
                p = jnp.exp2(sB[z2, c * KC:(c + 1) * KC, :] - mcur).astype(BF16)
                acc = pv(h2, c, p, acc)
                if c >= 2 and c - 2 < len(tasks):
                    t = pltpu.bitcast(tasks[c - 2]() | U32(0xff800000), F32)
                    m = jnp.concatenate([jnp.maximum(m[:, :128], t), m[:, 128:]], axis=1)
            if h1 is not None:
                mA[0:1, :] = jnp.max(m, axis=0, keepdims=True)
            finish(acc, h2 >> 1, h2 & 1, q2)

        def body(h, carry):
            g = (h * 43) >> 8
            z1 = h >> 10
            z2 = h >> 11
            for qi in range(NQ):
                if qi == 0:
                    fused(h, g, 0, jnp.maximum(h - 1, 0), NQ - 1, z1, z2, mac_tasks(h >> 1, h & 1, qi))
                else:
                    fused(h, g, qi, h, qi - 1, z1, z2, mac_tasks(h >> 1, h & 1, qi))
            return carry

        lax.fori_loop(0, H, body, 0)
        fused(None, None, 0, jnp.int32(H - 1), NQ - 1, 0, 0, [])

    def fast_path():
        def make_kb(h, kb, ds, z, gate=None):
            g = (h * 43) >> 8
            j = h - 6 * g
            o = (KC - 16) // 2 if VLAST else 0
            kk = jnp.concatenate([kk_s[g, c * KC // 2 + o:c * KC // 2 + o + 8, :] for c in VCH], axis=0)
            for d in ds:
                idx = jnp.full((8, 128), DH * j + d, jnp.int32)
                if gate is not None:
                    idx = idx + pltpu.bitcast(zero_bits(_u32(gate)), jnp.int32)
                idx = jnp.concatenate([idx] * len(VCH), axis=0)
                col = _bf(jnp.take_along_axis(kk, idx, axis=1)).astype(F32)
                kb[0, :, d] = col.reshape(len(VCH), 16, 128)
            if z is None:
                return None
            return zero_bits(_u32(kb[z, 0, 0, 0:8, :]))

        def add_at(s, r, t, z):
            row = s[8 * r:8 * r + 8]
            parts = [row[:, 128 * u:128 * (u + 1)] + z if u == t else row[:, 128 * u:128 * (u + 1)] for u in range(NT)]
            rows = ([s[:8 * r]] if r > 0 else []) + [jnp.concatenate(parts, axis=1)] + [s[8 * r + 8:]]
            return jnp.concatenate(rows, axis=0)

        def vpu_scores(i, h, kb, qi, c):
            v = VCH.index(c)
            hq = h + (i >> (10 + c))
            cols = []
            for t in range(NT):
                zz = i >> (10 + qi * NT + t)
                acc = None
                for d in range(DH):
                    qb = jnp.broadcast_to(qf_s[hq, d:d + 1, qi * TQ + t * 128:qi * TQ + (t + 1) * 128], (8, 128))
                    pr = kb[zz, v, d] * jnp.concatenate([qb, qb], axis=0)
                    acc = pr if acc is None else acc + pr
                cols.append(acc)
            return cols

        def body(i, carry):
            pend = []
            accs = {}
            toks = {}

            def drain():
                par, qi, c, p = pend.pop(0)
                accs[qi] = pv(2 * i + par, c, p, accs.get(qi))
                if c == NC - 1:
                    finish(accs.pop(qi), i, par, qi)

            steps = [(par, qi, c) for par in range(2) for qi in range(NQ) for c in range(NC)]
            use = [c in VCH and n >= SKIP0 for n, (par, qi, c) in enumerate(steps)]

            def sv_of(n):
                par, qi, c = steps[n]
                return vpu_scores(i, 2 * i + par, kb_s[par], qi, c)

            sv = {}
            if use[0]:
                sv[0] = sv_of(0)
            for step, (par, qi, c) in enumerate(steps):
                h = 2 * i + par
                g = (h * 43) >> 8
                hn = jnp.minimum(h + 1, H - 1)
                tasks = mac_tasks(i, par, qi)
                lo, hi = c * KC, (c + 1) * KC
                if use[step]:
                    if VLAST:
                        hi -= 16
                    else:
                        lo += 16
                s = jnp.dot(_bf(kk_s[g, lo // 2:hi // 2, :]),
                            _bf(qt_s[h, :, qi * TQ:(qi + 1) * TQ]), preferred_element_type=F32)
                gate = s[0:8, 0:128]
                if step in toks:
                    s = add_at(s, MROW, 0, pltpu.bitcast(toks.pop(step), F32))
                if step + 1 < len(steps) and use[step + 1]:
                    sv[step + 1] = sv_of(step + 1)
                    for t in range(NT):
                        a = sv[step + 1][t]
                        s = add_at(s, VROW[t], t, (a[0:8] + a[8:16]) * 0.0)
                s = unrev(s)
                if use[step]:
                    x = jnp.concatenate(sv.pop(step), axis=1)
                    s = jnp.concatenate([x, s] if VLAST else [s, x], axis=0)
                pend.append((par, qi, c, jnp.exp2(s).astype(BF16)))
                if len(pend) > LAG:
                    drain()
                new_toks = []
                if c < len(tasks):
                    if GATE:
                        w_s[i >> (10 + (step % 16)), 0, 66] = gate
                    new_toks.append(tasks[c]())
                n = qi * NC + c
                if VCH and n >= KB0 and (n - KB0) % KBS == 0 and (n - KB0) // KBS < DH:
                    d = (n - KB0) // KBS
                    t2 = make_kb(hn, kb_s[1 - par], [d], (i >> (10 + d)) if KANCH else None, gate if GATE else None)
                    if KANCH:
                        new_toks.append(t2)
                if ANCH and step + ANCH < len(steps):
                    for t in new_toks:
                        toks[step + ANCH] = t if step + ANCH not in toks else toks[step + ANCH] | t
            while pend:
                drain()
            return carry

        if VCH:
            make_kb(0, kb_s[0], range(DH), None)
        lax.fori_loop(0, H // 2, body, 0)

    qmax = jnp.max(mx_s[0])
    kmax = jnp.max(mx_s[1])
    vmax = jnp.max(mx_s[2])
    safe = (qmax * kmax * DH <= 72.0) & (vmax <= 2.0 ** 30) & (vmax >= 2.0 ** -30)
    if FORCE == "slow":
        slow_path()
    elif FORCE == "fast":
        fast_path()
    else:
        pl.when(safe)(fast_path)
        pl.when(jnp.logical_not(safe))(slow_path)

    cp_wo.wait()

    def out_copy(i):
        rows = pl.ds(pl.multiple_of(i * XC, XC), XC)
        return pltpu.make_async_copy(out_v.at[rows, :], out_hbm.at[0, rows, :], sem_o.at[i])

    def epilogue(i, carry):
        r0 = pl.multiple_of(i * XC, XC)
        rows = pl.ds(r0, XC)
        o = ot_s[:, rows].T.astype(BF16)
        bres = jnp.dot(o, wo_v[...], preferred_element_type=F32)
        inv = inv_ref[...]
        ys = []
        for bb in range(BPC):
            ys.append(jnp.dot(inv, _bf(y_s[i * BPC + bb]), preferred_element_type=F32))
        y = jnp.concatenate(ys, axis=0)
        x = x_v[rows, :].astype(F32)
        y = y + kv_s[rows, :].astype(F32) * dvec_ref[...].astype(F32)
        a = x * y
        logit = jnp.sum(x * gw_ref[...].astype(F32), axis=-1, keepdims=True)
        gate = jax.nn.sigmoid(logit)
        out_v[rows, :] = (bres + gate * (a - bres)).astype(BF16)
        out_copy(i).start()
        return carry

    lax.fori_loop(0, NX, epilogue, 0)
    for i in range(NX):
        out_copy(i).wait()


@jax.jit
def pallas_gated_mix__ssm_conv_h3__mha_block__prompt_kernel(
    A_q, A_k, A_v, A_shift_k, A_ssm_k, A_ssm_D, B_x, B_wqkv, B_wo, gate_w,
):
    del B_x
    fwd, inv = _dft_consts()
    any_spec = pl.BlockSpec(memory_space=pl.ANY)
    vm = pl.BlockSpec(memory_space=pltpu.VMEM)
    scratch = [
        pltpu.VMEM((S, D), BF16),
        pltpu.VMEM((S, D), BF16),
        pltpu.VMEM((S, D), BF16),
        pltpu.VMEM((D, S), BF16),
        pltpu.VMEM((D, 3 * D), BF16),
        pltpu.VMEM((D, D), BF16),
        pltpu.VMEM((S, D), BF16),
        pltpu.VMEM((D, NG * 128), BF16),
        pltpu.VMEM((2 * D, D), BF16),
        pltpu.VMEM((H, 64, S), U32),
        pltpu.VMEM((NG, S // 2, 128), U32),
        pltpu.VMEM((H, 16, S), U32),
        pltpu.VMEM((1, S, TQ), F32),
        pltpu.VMEM((1, S, TQ), F32),
        pltpu.VMEM((8, TQ), F32),
        pltpu.VMEM((8, TQ), F32),
        pltpu.VMEM((D, S), F32),
        pltpu.VMEM((16, 5, 68, 8, 128), F32),
        pltpu.VMEM((2 * B, D), F32),
        pltpu.VMEM((NB, B, D), U32),
        pltpu.VMEM((S, D), BF16),
        pltpu.VMEM((XC + 32, D), F32),
        pltpu.VMEM((H, 24, S), F32),
        pltpu.VMEM((4, 8, 128), F32),
        pltpu.SemaphoreType.DMA((2,)),
        pltpu.SemaphoreType.DMA((4 * NX,)),
        pltpu.SemaphoreType.DMA((NX,)),
    ] + [pltpu.VMEM((1, max(NVB, 1), DH, 16, 128), F32) for _ in range(2)]
    return pl.pallas_call(
        _kernel,
        out_shape=jax.ShapeDtypeStruct((1, S, D), BF16),
        in_specs=[any_spec] * 6 + [vm] * 5,
        out_specs=any_spec,
        scratch_shapes=scratch,
        compiler_params=pltpu.CompilerParams(vmem_limit_bytes=120 * 2 ** 20),
    )(A_q, A_k, A_v, A_ssm_k, B_wqkv, B_wo,
      A_shift_k.T, A_ssm_D.reshape(1, D), gate_w.reshape(1, D),
      jnp.asarray(fwd, BF16), jnp.asarray(inv, BF16))
```

```python
import math
import os as _os_

import numpy as np
import jax
import jax.numpy as jnp
from jax import lax
import jax.experimental.pallas as pl
import jax.experimental.pallas.tpu as pltpu

S = 2048
D = 640
H = 32
DH = 20
ND = D // 128
TQ = 512
NQ = S // TQ
NT = TQ // 128
KC = 128
NC = S // KC
B = 128
NB = S // B
XC = 512
NX = S // XC
BPC = XC // B
CC = int(_os_.environ.get("CC", "256"))
NCC = S // CC
NVB = int(_os_.environ.get("NVB", "20"))
KB0 = int(_os_.environ.get("KB0", "2"))
KBS = int(_os_.environ.get("KBS", "3"))
LOOK = int(_os_.environ.get("LOOK", "4"))
R0 = int(_os_.environ.get("R0", "0"))
R1 = int(_os_.environ.get("R1", "0"))
SH = int(_os_.environ.get("SH", "1"))
JL = int(_os_.environ.get("JL", "14"))
LA = int(_os_.environ.get("LA", "2"))
WI = int(_os_.environ.get("WI", "6"))
XI = int(_os_.environ.get("XI", "7"))
FORCE = _os_.environ.get("FORCE", "")
NV = [((c + 1) * NVB) // NC - (c * NVB) // NC for c in range(NC)][::-1]
VBLK = [(c, e) for c in range(NC) for e in range(NV[c])]

F32 = jnp.float32
BF16 = jnp.bfloat16
U32 = jnp.uint32


def _dft_consts():
    r = np.arange(2 * B)
    t, part, i = r // 16, (r // 8) % 2, r % 8
    f = np.where(t < 8, 2 * (8 * t + i), 2 * (8 * (t - 8) + i) + 1)
    theta = np.pi * (2 * f + 1) / (2 * B)
    j = np.arange(B)
    ang = theta[:, None] * j[None, :]
    fwd = np.where(part[:, None] == 0, np.cos(ang), -np.sin(ang))
    inv = fwd.T / B
    return fwd.astype(np.float32), inv.astype(np.float32)


def _bf(x):
    return pltpu.bitcast(x, BF16)


def _u32(x):
    return pltpu.bitcast(x, U32)


def _zero_bits(u):
    return lax.shift_right_logical(lax.shift_right_logical(u, U32(31)), U32(1))


def _add_tiles(s, adds):
    if not adds:
        return s
    rows = []
    done = 0
    for r in sorted({r for r, _ in adds}):
        if 8 * r > done:
            rows.append(s[done:8 * r])
        row = s[8 * r:8 * r + 8]
        parts = []
        cdone = 0
        for t in sorted(t for rr, t in adds if rr == r):
            if 128 * t > cdone:
                parts.append(row[:, cdone:128 * t])
            parts.append(row[:, 128 * t:128 * (t + 1)] + adds[(r, t)])
            cdone = 128 * (t + 1)
        if cdone < s.shape[1]:
            parts.append(row[:, cdone:])
        rows.append(jnp.concatenate(parts, axis=1))
        done = 8 * r + 8
    if done < s.shape[0]:
        rows.append(s[done:])
    return jnp.concatenate(rows, axis=0)


def _kernel(x_hbm, k_hbm, v_hbm, ssm_hbm, wqkv_hbm, wo_hbm,
            shift_ref, dvec_ref, gw_ref, fwd_ref, inv_ref,
            out_hbm,
            x_v, k_v, v_v, ssm_v, wqkv_v, wo_v, out_v,
            qt_s, kk_s, vt_s, s0, s1, m0, m1, ot_s,
            w_s, kf_s, y_s, kpad_s, qf_s, mx_s, kb0, kb1,
            sem_w, sem_x, sem_c, sem_o):
    kb_s = (kb0, kb1)
    cp_wqkv = pltpu.make_async_copy(wqkv_hbm, wqkv_v, sem_w.at[0])
    cp_wo = pltpu.make_async_copy(wo_hbm, wo_v, sem_w.at[1])

    def x_copy(i):
        rows = pl.ds(pl.multiple_of(i * XC, XC), XC)
        return pltpu.make_async_copy(x_hbm.at[0, rows, :], x_v.at[rows, :], sem_x.at[i])

    def conv_copies(i):
        rows = pl.ds(pl.multiple_of(i * CC, CC), CC)
        return [
            pltpu.make_async_copy(ssm_hbm.at[:, rows], ssm_v.at[:, rows], sem_c.at[3 * i]),
            pltpu.make_async_copy(k_hbm.at[0, rows, :], k_v.at[rows, :], sem_c.at[3 * i + 1]),
            pltpu.make_async_copy(v_hbm.at[0, rows, :], v_v.at[rows, :], sem_c.at[3 * i + 2]),
        ]

    for n in range(LA):
        for c in conv_copies(n):
            c.start()

    kf_s[...] = jnp.zeros((2 * B, D), F32)
    kpad_s[:, 0:8, :] = jnp.zeros((ND, 8, 128), F32)
    mx_s[...] = jnp.zeros_like(mx_s)

    def conv_phase(i, carry):
        for c in conv_copies(i):
            c.wait()

        @pl.when(i + LA < NCC)
        def _():
            for c in conv_copies(i + LA):
                c.start()

        @pl.when(i == WI)
        def _():
            cp_wqkv.start()

        @pl.when(i == XI)
        def _():
            x_copy(0).start()

        r0 = pl.multiple_of(i * CC, CC)
        sh = shift_ref[...].astype(F32)
        for dt in range(ND):
            kpad_s[dt, 8:8 + CC, :] = k_v[pl.ds(r0, CC), dt * 128:(dt + 1) * 128].astype(F32)
        fwd = fwd_ref[...]
        fwd32 = fwd.astype(F32)
        dterm = dvec_ref[...].astype(F32).reshape(1, D) * (i == 0).astype(F32)
        prev = kf_s[...].reshape(16, 2, 8, D)
        for bb in range(CC // B):
            b = i * (CC // B) + bb
            blk = pl.ds(pl.multiple_of(r0 + bb * B, B), B)
            kc = lax.dot_general(fwd, ssm_v[:, blk], (((1,), (1,)), ((), ())), preferred_element_type=F32)
            cur = kc.reshape(16, 2, 8, D)
            if bb == 0:
                cur = jnp.stack([cur[:, 0] + dterm, cur[:, 1]], axis=1)
            re = jnp.concatenate([cur[:8, 0] - prev[:8, 1], cur[8:, 0] + prev[8:, 1]], axis=0)
            im = jnp.concatenate([cur[:8, 1] + prev[:8, 0], cur[8:, 1] - prev[8:, 0]], axis=0)
            kp = jnp.stack([re, im], axis=1)
            for dt in range(ND):
                w_s[:, dt, pl.ds(4 * b, 2)] = kp[:, :, :, dt * 128:(dt + 1) * 128]
            prev = cur
            cols = []
            for dt in range(ND):
                ln = slice(dt * 128, (dt + 1) * 128)
                ks = None
                for l in range(4):
                    t = kpad_s[dt, 8 - l + bb * B:8 - l + (bb + 1) * B, :] * sh[l:l + 1, ln]
                    ks = t if ks is None else ks + t
                cols.append(ks * v_v[blk, ln].astype(F32))
            ub = jnp.dot(fwd32, jnp.concatenate(cols, axis=1), preferred_element_type=F32)
            ub = ub.reshape(16, 2, 8, D)
            for dt in range(ND):
                w_s[:, dt, pl.ds(4 * b + 2, 2)] = ub[:, :, :, dt * 128:(dt + 1) * 128]
        kpad_s[:, 0:8, :] = kpad_s[:, CC:CC + 8, :]
        kf_s[...] = prev.reshape(2 * B, D)
        return carry

    lax.fori_loop(0, NCC, conv_phase, 0)
    cp_wqkv.wait()

    qscale = (DH ** -0.5) * math.log2(math.e)

    def absmax8(a):
        a = jnp.abs(a)
        a = jnp.max(a.reshape(a.shape[0] // 8, 8, a.shape[1]), axis=0)
        r = a[:, 0:128]
        for t in range(1, a.shape[1] // 128):
            r = jnp.maximum(r, a[:, t * 128:(t + 1) * 128])
        return r

    def mac_task(ft, a, dt, z):
        yr = None
        yi = None
        for b in range(a + 1):
            kr = w_s[ft + z, dt, 4 * (a - b)]
            ki = w_s[ft + z, dt, 4 * (a - b) + 1]
            ur = w_s[ft + z, dt, 4 * b + 2]
            ui = w_s[ft + z, dt, 4 * b + 3]
            tr = kr * ur - ki * ui
            ti = kr * ui + ki * ur
            yr = tr if yr is None else yr + tr
            yi = ti if yi is None else yi + ti
        yu = _u32(jnp.concatenate([yr, yi], axis=0).astype(BF16))
        y_s[a, pl.ds(pl.multiple_of(ft * 8, 8), 8), dt * 128:(dt + 1) * 128] = yu
        return pltpu.bitcast(_zero_bits(yu), F32)

    def proj_phase(i, carry):
        x_copy(i).wait()

        @pl.when(i + 1 < NX)
        def _():
            x_copy(i + 1).start()

        rows = pl.ds(pl.multiple_of(i * XC, XC), XC)
        qkv = jnp.dot(x_v[rows, :], wqkv_v[...], preferred_element_type=F32)
        order = [a for p in range(NB // 2) for a in (p, NB - 1 - p)]
        tasks = [(f, a, dt) for f in range(16 // NX) for dt in range(ND) for a in order]
        adds = {}
        for n, (f, a, dt) in enumerate(tasks):
            pos = (n * JL * (XC // 8)) // len(tasks)
            adds[(pos % (XC // 8), pos // (XC // 8))] = mac_task(i * (16 // NX) + f, a, dt, i >> (10 + a))
        qkv = _add_tiles(qkv, adds)

        kf = qkv[:, D:2 * D]
        mx_s[1] = jnp.maximum(mx_s[1], absmax8(kf))
        kf = jnp.concatenate([kf[cc * KC + 8 * e:cc * KC + 8 * e + 8]
                              for cc in range(XC // KC) for e in reversed(range(KC // 8))], axis=0)
        kk = _u32(kf.astype(BF16))
        hrows = pl.ds(pl.multiple_of(i * (XC // 2), XC // 2), XC // 2)
        lane = lax.broadcasted_iota(jnp.int32, (XC // 2, 128), 1)
        qs = qkv[:, 0:D] * qscale
        vv = qkv[:, 2 * D:3 * D]
        mx_s[0] = jnp.maximum(mx_s[0], absmax8(qs))
        mx_s[2] = jnp.maximum(mx_s[2], absmax8(vv))
        qs = qs.T
        vv = vv.T
        row8 = lax.broadcasted_iota(jnp.int32, (8, XC), 0)
        for h in range(H):
            w = (DH * h) // 8 * 8
            t0, off = w // 128, w % 128
            kh = kk[:, t0 * 128:(t0 + 1) * 128]
            if off:
                kh = pltpu.roll(kh, 128 - off, 1)
            if off + 24 > 128:
                k2 = pltpu.roll(kk[:, (t0 + 1) * 128:(t0 + 2) * 128], 128 - off, 1)
                kh = jnp.where(lane < 128 - off, kh, k2)
            kk_s[h, hrows, :] = kh
            if h == 0:
                nvx = NVB // NX
                src = jnp.concatenate([kh[c * KC // 2 + 8 * e:c * KC // 2 + 8 * e + 8] for c, e in VBLK[:nvx]], axis=0)
                for d in range(DH):
                    col = _bf(jnp.broadcast_to(src[:, d:d + 1], src.shape)).astype(F32)
                    kb0[0, pl.ds(i * nvx, nvx), d] = col.reshape(nvx, 16, 128)
            qw = qs[w:w + 24, :]
            vw = vv[w:w + 24, :]
            qf_s[h, :, rows] = qw
            if h % 2 == 0:
                qparts = [qw[0:16], jnp.where(row8 < 4, qw[16:24], 0.0)]
                vparts = [vw[0:16], jnp.where(row8 == 4, 1.0, vw[16:24])]
            else:
                qparts = [jnp.where(row8 >= 4, qw[0:8], 0.0), qw[8:24]]
                vparts = [jnp.where(row8 == 0, 1.0, vw[0:8]), vw[8:24]]
            qt = jnp.concatenate(qparts + [jnp.zeros((8, XC), F32)], axis=0)
            qt_s[h, :, rows] = _u32(qt.astype(BF16))
            vt_s[h, :, rows] = jnp.concatenate(vparts, axis=0)
        return carry

    lax.fori_loop(0, NX, proj_phase, 0)
    cp_wo.start()

    def unrev(s):
        return jnp.concatenate([s[8 * e:8 * e + 8] for e in reversed(range(s.shape[0] // 8))], axis=0)

    def finish(acc, hp, par, q2):
        if isinstance(par, int):
            den = acc[20:21, :] if par == 0 else acc[0:1, :]
        else:
            den = jnp.where(par == 0, acc[20:21, :], acc[0:1, :])
        o = acc * pl.reciprocal(den, approx=False)
        w = pl.multiple_of(hp * 40 + par * 16, 8)
        row = lax.broadcasted_iota(jnp.int32, (24, TQ), 0)
        msk = (row >= 4 * par) & (row < 4 * par + DH)
        pltpu.store(ot_s.at[pl.ds(w, 24), q2 * TQ:(q2 + 1) * TQ], o, mask=msk)

    def qk(h, qi, *ranges):
        lhs = jnp.concatenate([kk_s[h, lo // 2:hi // 2, :] for lo, hi in ranges if hi > lo], axis=0)
        return jnp.dot(_bf(lhs)[:, 0:32], _bf(qt_s[h, :, qi * TQ:(qi + 1) * TQ]), preferred_element_type=F32)

    def pv(h, c, p, acc):
        o = jnp.dot(vt_s[h, :, c * KC:(c + 1) * KC], p, preferred_element_type=F32)
        return o if acc is None else acc + o

    def slow_path():
        sb = [s0, s1]
        mb = [m0, m1]
        s1[...] = jnp.zeros_like(s1)
        m1[...] = jnp.zeros_like(m1)

        def fused(h1, q1, h2, q2, z1, z2):
            sA, mA = sb[q1 % 2], mb[q1 % 2]
            sB, mB = sb[q2 % 2], mb[q2 % 2]
            mcur = mB[0:1, :]
            m = None
            acc = None
            for c in range(NC):
                if h1 is not None:
                    s = qk(h1, q1, (c * KC, (c + 1) * KC))
                    sA[z1, c * KC:(c + 1) * KC, :] = unrev(s)
                    mc = jnp.max(s.reshape(KC // 8, 8, TQ), axis=0)
                    m = mc if m is None else jnp.maximum(m, mc)
                p = jnp.exp2(sB[z2, c * KC:(c + 1) * KC, :] - mcur)
                acc = pv(h2, c, p, acc)
            if h1 is not None:
                mA[0:1, :] = jnp.max(m, axis=0, keepdims=True)
            finish(acc, h2 >> 1, h2 & 1, q2)

        def body(h, carry):
            z1 = h >> 10
            z2 = h >> 11
            fused(h, 0, jnp.maximum(h - 1, 0), NQ - 1, z1, z2)
            for qi in range(1, NQ):
                fused(h, qi, h, qi - 1, z1, z2)
            return carry

        lax.fori_loop(0, H, body, 0)
        fused(None, 0, jnp.int32(H - 1), NQ - 1, 0, 0)

    def fast_path():
        def make_kb(h, par, ds, gate=None):
            kk = jnp.concatenate([kk_s[h, c * KC // 2 + 8 * e:c * KC // 2 + 8 * e + 8, :] for c, e in VBLK], axis=0)
            for d in ds:
                idx = jnp.full((8, 128), 4 * par + d, jnp.int32)
                if gate is not None:
                    idx = idx + pltpu.bitcast(_zero_bits(_u32(gate)), jnp.int32)
                idx = jnp.concatenate([idx] * len(VBLK), axis=0)
                col = _bf(jnp.take_along_axis(kk, idx, axis=1)).astype(F32)
                kb_s[par][0, :, d] = col.reshape(len(VBLK), 16, 128)

        def vpu_chain(i, par, qi, c, e, t):
            v = VBLK.index((c, e))
            hq = 2 * i + par + (i >> (8 + v))
            zz = i >> (10 + qi * NT + t)
            acc = None
            for d in range(DH):
                qb = jnp.broadcast_to(
                    qf_s[hq, 4 * par + d:4 * par + d + 1, qi * TQ + t * 128:qi * TQ + (t + 1) * 128], (8, 128))
                pr = kb_s[par][zz, v, d] * jnp.concatenate([qb, qb], axis=0)
                acc = pr if acc is None else acc + pr
            return acc

        def body(i, carry):
            steps = [(par, qi, c) for par in range(2) for qi in range(NQ) for c in range(NC)]
            nv = [NV[c] if n >= 1 else 0 for n, (par, qi, c) in enumerate(steps)]
            queue = [(n, e, t) for n in range(len(steps)) for e in range(nv[n]) for t in range(NT)]
            quota = -(-NVB * NT // NC)
            sv = {}
            early = None
            pend = None
            acc = None

            def drain(acc):
                par, qi, c, p = pend
                acc = pv(2 * i + par, c, p, acc)
                if c == NC - 1:
                    finish(acc, i, par, qi)
                    acc = acc * 0.0
                return acc

            for step, (par, qi, c) in enumerate(steps):
                h = 2 * i + par
                lo = c * KC + 16 * nv[step] + (16 * SH if c > 0 else 0)
                lo2 = (c + 1) * KC + 16 * nv[step + 1] if c + 1 < NC else 0
                n2 = 16 * SH if c + 1 < NC else 0
                s = qk(h, qi, (lo, (c + 1) * KC), (lo2, lo2 + n2))
                gate = s[0:8, 0:128]
                todo = []
                while queue and (queue[0][0] <= step + 1 or
                                 (len(todo) < quota and queue[0][0] <= step + LOOK and steps[queue[0][0]][0] == par)):
                    todo.append(queue.pop(0))
                nrow = s.shape[0] // 8
                adds = {}
                for k, (n, e, t) in enumerate(todo):
                    a = vpu_chain(i, steps[n][0], steps[n][1], steps[n][2], e, t)
                    sv[(n, e, t)] = a
                    adds[(R0 + (k * (nrow - R0 - R1)) // len(todo), k % NT)] = (a[0:8] + a[8:16]) * 0.0
                s = _add_tiles(s, adds)
                x = [jnp.concatenate([sv.pop((step, e, t)) for t in range(NT)], axis=1) for e in range(nv[step])]
                if early is not None:
                    x.append(early)
                early = None
                if n2:
                    early = s[s.shape[0] - n2:]
                    s = s[:s.shape[0] - n2]
                p = jnp.exp2(unrev(jnp.concatenate(x + [s], axis=0)))
                if pend is not None:
                    acc = drain(acc)
                pend = (par, qi, c, p)
                n = qi * NC + c
                if n >= KB0 and (n - KB0) % KBS == 0 and (n - KB0) // KBS < DH:
                    hn = jnp.minimum(h + 1, H - 2) if par else h + 1
                    make_kb(hn, 1 - par, [(n - KB0) // KBS], gate)
            drain(acc)
            return carry

        lax.fori_loop(0, H // 2, body, 0)

    qmax = jnp.max(mx_s[0])
    kmax = jnp.max(mx_s[1])
    vmax = jnp.max(mx_s[2])
    safe = (qmax * kmax * DH <= 72.0) & (vmax <= 2.0 ** 30) & (vmax >= 2.0 ** -30)
    if FORCE == "none":
        ot_s[...] = jnp.zeros_like(ot_s)
    elif FORCE == "slow":
        slow_path()
    elif FORCE == "fast":
        fast_path()
    else:
        pl.when(safe)(fast_path)
        pl.when(jnp.logical_not(safe))(slow_path)

    cp_wo.wait()

    def out_copy(i):
        rows = pl.ds(pl.multiple_of(i * XC, XC), XC)
        return pltpu.make_async_copy(out_v.at[rows, :], out_hbm.at[0, rows, :], sem_o.at[i])

    def epilogue(i, carry):
        rows = pl.ds(pl.multiple_of(i * XC, XC), XC)
        inv = inv_ref[...]
        y = jnp.concatenate([jnp.dot(inv, _bf(y_s[i * BPC + bb]), preferred_element_type=F32)
                             for bb in range(BPC)], axis=0)
        o = ot_s[:, rows].T.astype(BF16)
        bres = jnp.dot(o, wo_v[...], preferred_element_type=F32)
        x = x_v[rows, :].astype(F32)
        logit = jnp.sum(x * gw_ref[...].astype(F32).reshape(1, D), axis=-1, keepdims=True)
        gate = jax.nn.sigmoid(logit)
        out_v[rows, :] = (bres + gate * (x * y - bres)).astype(BF16)
        out_copy(i).start()
        return carry

    lax.fori_loop(0, NX, epilogue, 0)
    for i in range(NX):
        out_copy(i).wait()


@jax.jit
def pallas_gated_mix__ssm_conv_h3__mha_block__prompt_kernel(
    A_q, A_k, A_v, A_shift_k, A_ssm_k, A_ssm_D, B_x, B_wqkv, B_wo, gate_w,
):
    del B_x
    fwd, inv = _dft_consts()
    any_spec = pl.BlockSpec(memory_space=pl.ANY)
    vm = pl.BlockSpec(memory_space=pltpu.VMEM)
    scratch = [
        pltpu.VMEM((S, D), BF16),
        pltpu.VMEM((S, D), BF16),
        pltpu.VMEM((S, D), BF16),
        pltpu.VMEM((D, S), BF16),
        pltpu.VMEM((D, 3 * D), BF16),
        pltpu.VMEM((D, D), BF16),
        pltpu.VMEM((S, D), BF16),
        pltpu.VMEM((H, 16, S), U32),
        pltpu.VMEM((H, S // 2, 128), U32),
        pltpu.VMEM((H, 24, S), F32),
        pltpu.VMEM((1, S, TQ), F32),
        pltpu.VMEM((1, S, TQ), F32),
        pltpu.VMEM((8, TQ), F32),
        pltpu.VMEM((8, TQ), F32),
        pltpu.VMEM((D, S), F32),
        pltpu.VMEM((16, ND, 4 * NB, 8, 128), F32),
        pltpu.VMEM((2 * B, D), F32),
        pltpu.VMEM((NB, B, D), U32),
        pltpu.VMEM((ND, CC + 32, 128), F32),
        pltpu.VMEM((H, 24, S), F32),
        pltpu.VMEM((4, 8, 128), F32),
        pltpu.VMEM((1, NVB, DH, 16, 128), F32),
        pltpu.VMEM((1, NVB, DH, 16, 128), F32),
        pltpu.SemaphoreType.DMA((2,)),
        pltpu.SemaphoreType.DMA((NX,)),
        pltpu.SemaphoreType.DMA((3 * NCC,)),
        pltpu.SemaphoreType.DMA((NX,)),
    ]
    return pl.pallas_call(
        _kernel,
        out_shape=jax.ShapeDtypeStruct((1, S, D), BF16),
        in_specs=[any_spec] * 6 + [vm] * 5,
        out_specs=any_spec,
        scratch_shapes=scratch,
        compiler_params=pltpu.CompilerParams(vmem_limit_bytes=120 * 2 ** 20),
    )(A_q, A_k, A_v, A_ssm_k, B_wqkv, B_wo,
      A_shift_k.T, A_ssm_D, gate_w,
      jnp.asarray(fwd, BF16), jnp.asarray(inv, BF16))
```

```python
import math

import numpy as np
import jax
import jax.numpy as jnp
from jax import lax
import jax.experimental.pallas as pl
import jax.experimental.pallas.tpu as pltpu

S = 2048
D = 640
H = 32
DH = 20
ND = D // 128
TQ = 512
NQ = S // TQ
NT = TQ // 128
KC = 128
NC = S // KC
B = 128
NB = S // B
XC = 512
NX = S // XC
CC = 256
NCC = S // CC
LA = 3
EB = 5
NV = [2, 1, 1, 1] * (NC // 4)
NVB = sum(NV)
VBLK = [(c, e) for c in range(NC) for e in range(NV[c])]
JORD = [0, 1, 2, 3, 4, 5, 10, 11, 12, 13, 14, 6, 7, 8, 9]

F32 = jnp.float32
BF16 = jnp.bfloat16
U32 = jnp.uint32


def _dft_consts():
    r = np.arange(2 * B)
    t, part, i = r // 16, (r // 8) % 2, r % 8
    f = np.where(t < 8, 2 * (8 * t + i), 2 * (8 * (t - 8) + i) + 1)
    theta = np.pi * (2 * f + 1) / (2 * B)
    ang = theta[:, None] * np.arange(B)[None, :]
    fwd = np.where(part[:, None] == 0, np.cos(ang), -np.sin(ang))
    inv = fwd.T / B
    return fwd.astype(np.float32), inv.astype(np.float32)


def _bf(x):
    return pltpu.bitcast(x, BF16)


def _u32(x):
    return pltpu.bitcast(x, U32)


def _dot(a, b):
    return jnp.dot(a, b, precision=lax.Precision.DEFAULT, preferred_element_type=F32)


def _zero_bits(u):
    return lax.shift_right_logical(lax.shift_right_logical(u, U32(31)), U32(1))


def _add_tiles(s, adds):
    if not adds:
        return s
    rows = []
    done = 0
    for r in sorted({r for r, _ in adds}):
        if 8 * r > done:
            rows.append(s[done:8 * r])
        row = s[8 * r:8 * r + 8]
        parts = []
        cdone = 0
        for t in sorted(t for rr, t in adds if rr == r):
            if 128 * t > cdone:
                parts.append(row[:, cdone:128 * t])
            parts.append(row[:, 128 * t:128 * (t + 1)] + adds[(r, t)])
            cdone = 128 * (t + 1)
        if cdone < s.shape[1]:
            parts.append(row[:, cdone:])
        rows.append(jnp.concatenate(parts, axis=1))
        done = 8 * r + 8
    if done < s.shape[0]:
        rows.append(s[done:])
    return jnp.concatenate(rows, axis=0)


def _kernel(x_hbm, k_hbm, v_hbm, ssm_hbm, wqkv_hbm, wo_hbm,
            shift_hbm, dvec_hbm, gw_hbm, fwd_hbm, inv_hbm,
            out_hbm,
            fwd_ref, inv_ref, x_v, k_v, v_v, ssm_v, wqkv_v, wo_v, out_v,
            qt_s, kk_s, vt_s, s0, s1, m0, m1, ot_s,
            w_s, kf_s, y_s, kpad_s, qf_s, mx_s, kb0, kb1,
            shift_ref, dvec_ref, gw_ref,
            sem_w, sem_x, sem_c, sem_o, sem_s):
    kb_s = (kb0, kb1)
    cp_wqkv = pltpu.make_async_copy(wqkv_hbm, wqkv_v, sem_w.at[0])
    cp_wo = pltpu.make_async_copy(wo_hbm, wo_v, sem_w.at[1])

    def x_copy(i):
        rows = pl.ds(pl.multiple_of(i * XC, XC), XC)
        return pltpu.make_async_copy(x_hbm.at[0, rows, :], x_v.at[rows, :], sem_x.at[i])

    def conv_copies(i):
        rows = pl.ds(pl.multiple_of(i * CC, CC), CC)
        return [
            pltpu.make_async_copy(ssm_hbm.at[:, rows], ssm_v.at[:, rows], sem_c.at[3 * i]),
            pltpu.make_async_copy(k_hbm.at[0, rows, :], k_v.at[rows, :], sem_c.at[3 * i + 1]),
            pltpu.make_async_copy(v_hbm.at[0, rows, :], v_v.at[rows, :], sem_c.at[3 * i + 2]),
        ]

    small = [pltpu.make_async_copy(src, dst, sem_s.at[n]) for n, (src, dst) in enumerate(
        [(fwd_hbm, fwd_ref), (shift_hbm, shift_ref), (dvec_hbm, dvec_ref), (gw_hbm, gw_ref), (inv_hbm, inv_ref)])]
    for c in conv_copies(0) + small:
        c.start()
    for n in range(1, LA):
        for c in conv_copies(n):
            c.start()

    kf_s[...] = jnp.zeros((2 * B, D), F32)
    kpad_s[:, 0:8, :] = jnp.zeros((ND, 8, 128), F32)
    mx_s[...] = jnp.zeros_like(mx_s)
    ot_s[...] = jnp.zeros_like(ot_s)
    for h in range(H):
        qt_s[h, 16 - 16 * (h % 2):24 - 16 * (h % 2), :] = jnp.zeros((8, S), U32)
    for c in small:
        c.wait()

    def conv_phase(i, carry):
        for c in conv_copies(i):
            c.wait()

        @pl.when(i + LA < NCC)
        def _():
            for c in conv_copies(i + LA):
                c.start()

        @pl.when(i == NCC - LA)
        def _():
            cp_wqkv.start()

        @pl.when(i == NCC - LA + 1)
        def _():
            x_copy(0).start()

        r0 = pl.multiple_of(i * CC, CC)
        sh = shift_ref[...].astype(F32)
        for dt in range(ND):
            kpad_s[dt, 8:8 + CC, :] = k_v[pl.ds(r0, CC), dt * 128:(dt + 1) * 128].astype(F32)
        fwd = fwd_ref[...]
        fwd32 = fwd.astype(F32)
        dterm = dvec_ref[...].astype(F32).reshape(1, D) * (i == 0).astype(F32)
        prev = kf_s[...].reshape(16, 2, 8, D)
        for bb in range(CC // B):
            b = i * (CC // B) + bb
            blk = pl.ds(pl.multiple_of(r0 + bb * B, B), B)
            kc = lax.dot_general(fwd, ssm_v[:, blk], (((1,), (1,)), ((), ())), preferred_element_type=F32)
            cur = kc.reshape(16, 2, 8, D)
            if bb == 0:
                cur = jnp.stack([cur[:, 0] + dterm, cur[:, 1]], axis=1)
            re = jnp.concatenate([cur[:8, 0] - prev[:8, 1], cur[8:, 0] + prev[8:, 1]], axis=0)
            im = jnp.concatenate([cur[:8, 1] + prev[:8, 0], cur[8:, 1] - prev[8:, 0]], axis=0)
            kp = jnp.stack([re, im], axis=1)
            for dt in range(ND):
                w_s[:, dt, pl.ds(4 * b, 2)] = kp[:, :, :, dt * 128:(dt + 1) * 128]
            prev = cur
            cols = []
            for dt in range(ND):
                ln = slice(dt * 128, (dt + 1) * 128)
                ks = None
                for l in range(4):
                    t = kpad_s[dt, 8 - l + bb * B:8 - l + (bb + 1) * B, :] * sh[l:l + 1, ln]
                    ks = t if ks is None else ks + t
                cols.append(ks * v_v[blk, ln].astype(F32))
            ub = _dot(fwd32, jnp.concatenate(cols, axis=1)).reshape(16, 2, 8, D)
            for dt in range(ND):
                w_s[:, dt, pl.ds(4 * b + 2, 2)] = ub[:, :, :, dt * 128:(dt + 1) * 128]
        kpad_s[:, 0:8, :] = kpad_s[:, CC:CC + 8, :]
        kf_s[...] = prev.reshape(2 * B, D)
        return carry

    lax.fori_loop(0, NCC, conv_phase, 0)
    cp_wqkv.wait()

    qscale = (DH ** -0.5) * math.log2(math.e)

    def absmax8(a):
        a = jnp.abs(a)
        a = jnp.max(a.reshape(a.shape[0] // 8, 8, a.shape[1]), axis=0)
        r = a[:, 0:128]
        for t in range(1, a.shape[1] // 128):
            r = jnp.maximum(r, a[:, t * 128:(t + 1) * 128])
        return r

    def mac_task(ft, a, dt, z):
        yr = None
        yi = None
        for b in range(a + 1):
            kr = w_s[ft + z, dt, 4 * (a - b)]
            ki = w_s[ft + z, dt, 4 * (a - b) + 1]
            ur = w_s[ft + z, dt, 4 * b + 2]
            ui = w_s[ft + z, dt, 4 * b + 3]
            tr = kr * ur - ki * ui
            ti = kr * ui + ki * ur
            yr = tr if yr is None else yr + tr
            yi = ti if yi is None else yi + ti
        y_s[a, dt, ft, 0] = yr
        y_s[a, dt, ft, 1] = yi
        return pltpu.bitcast(_zero_bits(_u32(yr) | _u32(yi)), F32)

    def proj_phase(i, carry):
        x_copy(i).wait()

        @pl.when(i + 1 < NX)
        def _():
            x_copy(i + 1).start()

        rows = pl.ds(pl.multiple_of(i * XC, XC), XC)
        order = [a for p in range(NB // 2) for a in (p, NB - 1 - p)]
        tasks = [(f, a, dt) for f in range(16 // NX) for dt in range(ND) for a in order]
        wts = [60 if rd >= 13 else 100 for rd in range((3 * ND * ND) // 4)]
        cum = np.cumsum([0] + wts)
        adds = {}
        for n, (f, a, dt) in enumerate(tasks):
            pos = (n + 0.5) * cum[-1] / len(tasks)
            rd = int(np.searchsorted(cum, pos, side="right")) - 1
            r = int((pos - cum[rd]) / wts[rd] * (XC // 8))
            adds.setdefault(4 * rd + n % 4, {})[(r, 0)] = mac_task(i * (16 // NX) + f, a, dt, i >> (10 + a))
        x = x_v[rows, :]
        cols = [None] * (3 * ND)
        for jj, j in enumerate(JORD):
            acc = None
            for k in range(ND):
                t = _dot(x[:, k * 128:(k + 1) * 128], wqkv_v[k * 128:(k + 1) * 128, j * 128:(j + 1) * 128])
                t = _add_tiles(t, adds.get(jj * ND + k))
                acc = t if acc is None else acc + t
            cols[j] = acc
        qkv = jnp.concatenate(cols, axis=1)

        kf = qkv[:, D:2 * D]
        mx_s[1] = jnp.maximum(mx_s[1], absmax8(kf))
        kf = jnp.concatenate([kf[cc * KC + 8 * e:cc * KC + 8 * e + 8]
                              for cc in range(XC // KC) for e in reversed(range(KC // 8))], axis=0)
        kk = _u32(kf.astype(BF16))
        hrows = pl.ds(pl.multiple_of(i * (XC // 2), XC // 2), XC // 2)
        lane = lax.broadcasted_iota(jnp.int32, (XC // 2, 128), 1)
        qs = qkv[:, 0:D] * qscale
        vv = qkv[:, 2 * D:3 * D]
        mx_s[0] = jnp.maximum(mx_s[0], absmax8(qs))
        mx_s[2] = jnp.maximum(mx_s[2], absmax8(vv))
        qs = qs.T
        vv = vv.T
        row8 = lax.broadcasted_iota(jnp.int32, (8, XC), 0)
        zrows = jnp.zeros((8, XC), F32)
        for h in range(H):
            w = (DH * h) // 8 * 8
            if h % 2 == 0:
                t0, off = w // 128, w % 128
                kh = kk[:, t0 * 128:(t0 + 1) * 128]
                if off:
                    kh = pltpu.roll(kh, 128 - off, 1)
                if off + 2 * DH > 128:
                    k2 = pltpu.roll(kk[:, (t0 + 1) * 128:(t0 + 2) * 128], 128 - off, 1)
                    kh = jnp.where(lane < 128 - off, kh, k2)
                kk_s[h // 2, hrows, :] = kh
            if h == 0:
                nvx = NVB // NX
                src = jnp.concatenate([kh[c * KC // 2 + 8 * e:c * KC // 2 + 8 * e + 8] for c, e in VBLK[:nvx]], axis=0)
                for d in range(DH):
                    col = _bf(jnp.broadcast_to(src[:, d:d + 1], src.shape)).astype(F32)
                    kb0[0, pl.ds(i * nvx, nvx), d] = col.reshape(nvx, 16, 128)
            qw = qs[w:w + 24, :]
            vw = vv[w:w + 24, :]
            qf_s[h, :, rows] = qw
            if h % 2 == 0:
                qparts = [qw[0:16], jnp.where(row8 < 4, qw[16:24], 0.0)]
                vparts = [vw[0:16], jnp.where(row8 == 4, 1.0, vw[16:24])]
            else:
                qparts = [jnp.where(row8 >= 4, qw[0:8], 0.0), qw[8:24]]
                vparts = [jnp.where(row8 == 0, 1.0, vw[0:8]), vw[8:24]]
            qt = _u32(jnp.concatenate(qparts + [zrows], axis=0).astype(BF16))
            qt_s[h, 8 * (h % 2):8 * (h % 2) + 16, rows] = qt
            vt_s[h, :, rows] = jnp.concatenate(vparts, axis=0)
        return carry

    lax.fori_loop(0, NX, proj_phase, 0)
    cp_wo.start()

    def unrev(s):
        return jnp.concatenate([s[8 * e:8 * e + 8] for e in reversed(range(s.shape[0] // 8))], axis=0)

    def finish(acc, hp, par, q2):
        if isinstance(par, int):
            den = acc[20:21, :] if par == 0 else acc[0:1, :]
        else:
            den = jnp.where(par == 0, acc[20:21, :], acc[0:1, :])
        o = acc * pl.reciprocal(den, approx=False)
        w = pl.multiple_of(hp * 40 + par * 16, 8)
        row = lax.broadcasted_iota(jnp.int32, (24, TQ), 0)
        msk = (row >= 4 * par) & (row < 4 * par + DH)
        pltpu.store(ot_s.at[pl.ds(w, 24), q2 * TQ:(q2 + 1) * TQ], o, mask=msk)

    def qk(hp, h, kd, qi, *ranges):
        lhs = jnp.concatenate([kk_s[hp, lo // 2:hi // 2, :] for lo, hi in ranges if hi > lo], axis=0)
        return _dot(_bf(lhs)[:, 0:kd], _bf(qt_s[h, 0:kd // 2, qi * TQ:(qi + 1) * TQ]))

    def pv(h, c, p, acc):
        o = _dot(vt_s[h, :, c * KC:(c + 1) * KC], p)
        return o if acc is None else acc + o

    def slow_path():
        sb = [s0, s1]
        mb = [m0, m1]
        s1[...] = jnp.zeros_like(s1)
        m1[...] = jnp.zeros_like(m1)

        def fused(h1, q1, h2, q2, z1, z2):
            sA, mA = sb[q1 % 2], mb[q1 % 2]
            sB, mB = sb[q2 % 2], mb[q2 % 2]
            mcur = mB[0:1, :]
            m = None
            acc = None
            for c in range(NC):
                if h1 is not None:
                    s = qk(h1 >> 1, h1, 48, q1, (c * KC, (c + 1) * KC))
                    sA[z1, c * KC:(c + 1) * KC, :] = unrev(s)
                    mc = jnp.max(s.reshape(KC // 8, 8, TQ), axis=0)
                    m = mc if m is None else jnp.maximum(m, mc)
                p = jnp.exp2(sB[z2, c * KC:(c + 1) * KC, :] - mcur)
                acc = pv(h2, c, p, acc)
            if h1 is not None:
                mA[0:1, :] = jnp.max(m, axis=0, keepdims=True)
            finish(acc, h2 >> 1, h2 & 1, q2)

        def body(h, carry):
            z1 = h >> 10
            z2 = h >> 11
            fused(h, 0, jnp.maximum(h - 1, 0), NQ - 1, z1, z2)
            for qi in range(1, NQ):
                fused(h, qi, h, qi - 1, z1, z2)
            return carry

        lax.fori_loop(0, H, body, 0)
        fused(None, 0, jnp.int32(H - 1), NQ - 1, 0, 0)

    def fast_path():
        def make_kb(hp, par, d, gate):
            z = _zero_bits(_u32(gate))
            kk = jnp.concatenate([kk_s[hp, c * KC // 2 + 8 * e:c * KC // 2 + 8 * e + 8, :] | z for c, e in VBLK],
                                 axis=0)
            col = _bf(jnp.broadcast_to(kk[:, DH * par + d:DH * par + d + 1], kk.shape)).astype(F32)
            kb_s[par][0, :, d] = col.reshape(NVB, 16, 128)

        def vpu_chain(i, par, qi, c, e, t):
            v = VBLK.index((c, e))
            hq = 2 * i + par + (i >> (8 + v))
            zz = i >> (10 + qi * NT + t)
            acc = None
            for d in range(DH):
                qb = jnp.broadcast_to(
                    qf_s[hq, 4 * par + d:4 * par + d + 1, qi * TQ + t * 128:qi * TQ + (t + 1) * 128], (8, 128))
                pr = kb_s[par][zz, v, d] * jnp.concatenate([qb, qb], axis=0)
                acc = pr if acc is None else acc + pr
            return acc

        def body(i, carry):
            steps = [(par, qi, c) for par in range(2) for qi in range(NQ) for c in range(NC)]
            nv = [NV[c] if n >= 1 else 0 for n, (par, qi, c) in enumerate(steps)]
            queue = [(n, e, t) for n in range(len(steps)) for e in range(nv[n]) for t in range(NT)]
            quota = NVB * NT // NC
            sv = {}
            early = None
            pend = None
            acc = None

            def drain(acc):
                par, qi, c, p = pend
                acc = pv(2 * i + par, c, p, acc)
                if c == NC - 1:
                    finish(acc, i, par, qi)
                    acc = acc * 0.0
                return acc

            for step, (par, qi, c) in enumerate(steps):
                lo = c * KC + 16 * nv[step] + (16 if c > 0 else 0)
                lo2 = (c + 1) * KC + 16 * nv[step + 1] if c + 1 < NC else 0
                n2 = 16 if c + 1 < NC else 0
                s = qk(i, 2 * i + par, 48 if par else 32, qi, (lo, (c + 1) * KC), (lo2, lo2 + n2))
                gate = s[0:8, 0:128]
                todo = []
                while queue and (queue[0][0] <= step + 1 or
                                 (len(todo) < quota and steps[queue[0][0]][0] == par)):
                    todo.append(queue.pop(0))
                adds = {}
                for k, (n, e, t) in enumerate(todo):
                    a = vpu_chain(i, steps[n][0], steps[n][1], steps[n][2], e, t)
                    sv[(n, e, t)] = a
                    adds[((k * (s.shape[0] // 8)) // len(todo), NT - 1)] = (a[0:8] + a[8:16]) * 0.0
                s = _add_tiles(s, adds)
                x = [jnp.concatenate([sv.pop((step, e, t)) for t in range(NT)], axis=1) for e in range(nv[step])]
                if early is not None:
                    x.append(early)
                early = None
                if n2:
                    early = s[s.shape[0] - n2:]
                    s = s[:s.shape[0] - n2]
                p = jnp.exp2(unrev(jnp.concatenate(x + [s], axis=0)))
                if pend is not None:
                    acc = drain(acc)
                pend = (par, qi, c, p)
                n = qi * NC + c
                if n % 3 == 1 and n // 3 < DH:
                    make_kb(jnp.minimum(i + 1, H // 2 - 1) if par else i, 1 - par, n // 3, gate)
            drain(acc)
            return carry

        lax.fori_loop(0, H // 2, body, 0)

    qmax = jnp.max(mx_s[0])
    kmax = jnp.max(mx_s[1])
    vmax = jnp.max(mx_s[2])
    safe = (qmax * kmax * DH <= 80.0) & (vmax <= 2.0 ** 30) & (vmax >= 2.0 ** -30)
    lax.cond(safe, fast_path, slow_path)

    cp_wo.wait()

    def out_copy(i, nb):
        rows = pl.ds(pl.multiple_of(i * EB * B, B), nb * B)
        return pltpu.make_async_copy(out_v.at[rows, :], out_hbm.at[0, rows, :], sem_o.at[i])

    def epilogue(i, nb):
        rows = pl.ds(pl.multiple_of(i * EB * B, B), nb * B)
        inv = inv_ref[...].astype(F32)
        ys = []
        for bb in range(nb):
            yf = jnp.concatenate([y_s[i * EB + bb, dt].reshape(2 * B, 128) for dt in range(ND)], axis=1)
            ys.append(_dot(inv, yf))
        y = jnp.concatenate(ys, axis=0)
        o = ot_s[:, rows].T.astype(BF16)
        adds = {}
        tiles = [(a, b) for a in range(nb) for b in range(ND)]
        for n, (a, b) in enumerate(tiles):
            z = _zero_bits(_u32(o[a * 128 + 112:a * 128 + 128, b * 128:(b + 1) * 128]))
            pos = (2 * len(tiles) + 10 * n) // 20
            adds[((pos // ND) * 16 + n % 16, pos % ND)] = pltpu.bitcast(z, F32)
        y = _add_tiles(y, adds)
        bres = _dot(o, wo_v[...])
        x = x_v[rows, :].astype(F32)
        logit = jnp.sum(x * gw_ref[...].astype(F32).reshape(1, D), axis=-1, keepdims=True)
        gate = jax.nn.sigmoid(logit)
        out_v[rows, :] = (bres + gate * (x * y - bres)).astype(BF16)
        out_copy(i, nb).start()

    def epilogue_body(i, carry):
        epilogue(i, EB)
        return carry

    ne = NB // EB
    lax.fori_loop(0, ne, epilogue_body, 0)
    epilogue(ne, NB % EB)
    for i in range(ne):
        out_copy(i, EB).wait()
    out_copy(ne, NB % EB).wait()


@jax.jit
def pallas_gated_mix__ssm_conv_h3__mha_block__prompt_kernel(
    A_q: jax.Array,
    A_k: jax.Array,
    A_v: jax.Array,
    A_shift_k: jax.Array,
    A_ssm_k: jax.Array,
    A_ssm_D: jax.Array,
    B_x: jax.Array,
    B_wqkv: jax.Array,
    B_wo: jax.Array,
    gate_w: jax.Array,
):
    del B_x
    fwd, inv = _dft_consts()
    any_spec = pl.BlockSpec(memory_space=pl.ANY)
    scratch = [
        pltpu.VMEM((2 * B, B), BF16),
        pltpu.VMEM((B, 2 * B), BF16),
        pltpu.VMEM((S, D), BF16),
        pltpu.VMEM((S, D), BF16),
        pltpu.VMEM((S, D), BF16),
        pltpu.VMEM((D, S), BF16),
        pltpu.VMEM((D, 3 * D), BF16),
        pltpu.VMEM((D, D), BF16),
        pltpu.VMEM((S, D), BF16),
        pltpu.VMEM((H, 24, S), U32),
        pltpu.VMEM((H // 2, S // 2, 128), U32),
        pltpu.VMEM((H, 24, S), F32),
        pltpu.VMEM((1, S, TQ), F32),
        pltpu.VMEM((1, S, TQ), F32),
        pltpu.VMEM((8, TQ), F32),
        pltpu.VMEM((8, TQ), F32),
        pltpu.VMEM((D, S), F32),
        pltpu.VMEM((16, ND, 4 * NB, 8, 128), F32),
        pltpu.VMEM((2 * B, D), F32),
        pltpu.VMEM((NB, ND, 16, 2, 8, 128), F32),
        pltpu.VMEM((ND, CC + 32, 128), F32),
        pltpu.VMEM((H, 24, S), F32),
        pltpu.VMEM((4, 8, 128), F32),
        pltpu.VMEM((1, NVB, DH, 16, 128), F32),
        pltpu.VMEM((1, NVB, DH, 16, 128), F32),
        pltpu.VMEM((4, D), BF16),
        pltpu.VMEM((D,), BF16),
        pltpu.VMEM((D,), BF16),
        pltpu.SemaphoreType.DMA((2,)),
        pltpu.SemaphoreType.DMA((NX,)),
        pltpu.SemaphoreType.DMA((3 * NCC,)),
        pltpu.SemaphoreType.DMA((NB // EB + 1,)),
        pltpu.SemaphoreType.DMA((5,)),
    ]
    return pl.pallas_call(
        _kernel,
        out_shape=jax.ShapeDtypeStruct((1, S, D), BF16),
        in_specs=[any_spec] * 11,
        out_specs=any_spec,
        scratch_shapes=scratch,
        compiler_params=pltpu.CompilerParams(vmem_limit_bytes=120 * 2 ** 20),
    )(A_q, A_k, A_v, A_ssm_k, B_wqkv, B_wo,
      A_shift_k.T, A_ssm_D, gate_w,
      jnp.asarray(fwd, BF16), jnp.asarray(inv, BF16))
```

```python
import math

import numpy as np
import jax
import jax.numpy as jnp
from jax import lax
import jax.experimental.pallas as pl
import jax.experimental.pallas.tpu as pltpu

S = 2048
D = 640
H = 32
DH = 20
ND = D // 128
TQ = 512
NQ = S // TQ
NT = TQ // 128
KC = 128
NC = S // KC
B = 128
NB = S // B
XC = 512
NX = S // XC
NPOS = 22
EB = 5
NV = [2, 1, 1, 1] * (NC // 4)
NVB = sum(NV)
VBLK = [(c, e) for c in range(NC) for e in range(NV[c])]
JORD = [0, 1, 2, 3, 4, 5, 10, 11, 12, 13, 14, 6, 7, 8, 9]

F32 = jnp.float32
BF16 = jnp.bfloat16
U32 = jnp.uint32


def _dft_consts():
    r = np.arange(2 * B)
    t, part, i = r // 16, (r // 8) % 2, r % 8
    f = np.where(t < 8, 2 * (8 * t + i), 2 * (8 * (t - 8) + i) + 1)
    theta = np.pi * (2 * f + 1) / (2 * B)
    ang = theta[:, None] * np.arange(B)[None, :]
    fwd = np.where(part[:, None] == 0, np.cos(ang), -np.sin(ang))
    inv = fwd.T / B
    return fwd.astype(np.float32), inv.astype(np.float32)


def _bf(x):
    return pltpu.bitcast(x, BF16)


def _u32(x):
    return pltpu.bitcast(x, U32)


def _dot(a, b):
    return jnp.dot(a, b, precision=lax.Precision.DEFAULT, preferred_element_type=F32)


def _zero_bits(u):
    return lax.shift_right_logical(lax.shift_right_logical(u, U32(31)), U32(1))


def _add_tiles(s, adds):
    if not adds:
        return s
    rows = []
    done = 0
    for r in sorted({r for r, _ in adds}):
        if 8 * r > done:
            rows.append(s[done:8 * r])
        row = s[8 * r:8 * r + 8]
        parts = []
        cdone = 0
        for t in sorted(t for rr, t in adds if rr == r):
            if 128 * t > cdone:
                parts.append(row[:, cdone:128 * t])
            parts.append(row[:, 128 * t:128 * (t + 1)] + adds[(r, t)])
            cdone = 128 * (t + 1)
        if cdone < s.shape[1]:
            parts.append(row[:, cdone:])
        rows.append(jnp.concatenate(parts, axis=1))
        done = 8 * r + 8
    if done < s.shape[0]:
        rows.append(s[done:])
    return jnp.concatenate(rows, axis=0)


def _kernel(x_hbm, k_hbm, v_hbm, ssm_hbm, wqkv_hbm, wo_hbm,
            shift_hbm, dvec_hbm, gw_hbm, fwd_hbm, inv_hbm,
            out_hbm,
            mx_s, fwd_ref, inv_ref, x_v, k_v, v_v, ssm_v, wqkv_v, wo_v, out_v,
            qt_s, kk_s, vt_s, s0, s1, m0, m1, ot_s,
            w_s, par_s, y_s, qf_s, kb0, kb1,
            sem_w, sem_x, sem_c, sem_o, sem_s):
    kb_s = (kb0, kb1)
    cp_wqkv = pltpu.make_async_copy(wqkv_hbm, wqkv_v, sem_w.at[0])
    cp_wo = pltpu.make_async_copy(wo_hbm, wo_v, sem_w.at[1])

    def x_copy(i):
        rows = pl.ds(pl.multiple_of(i * XC, XC), XC)
        return pltpu.make_async_copy(x_hbm.at[0, rows, :], x_v.at[rows, :], sem_x.at[i])

    def conv_copies(dt):
        ln = pl.ds(pl.multiple_of(dt * 128, 128), 128)
        return [
            pltpu.make_async_copy(ssm_hbm.at[ln, :], ssm_v.at[dt], sem_c.at[3 * dt]),
            pltpu.make_async_copy(k_hbm.at[0, :, ln], k_v.at[dt], sem_c.at[3 * dt + 1]),
            pltpu.make_async_copy(v_hbm.at[0, :, ln], v_v.at[dt], sem_c.at[3 * dt + 2]),
        ]

    def setup(shift_ref, dvec_ref, gw_ref):
        small = [pltpu.make_async_copy(src, dst, sem_s.at[n]) for n, (src, dst) in enumerate(
            [(shift_hbm, shift_ref), (dvec_hbm, dvec_ref), (gw_hbm, gw_ref), (fwd_hbm, fwd_ref), (inv_hbm, inv_ref)])]
        for c in small:
            c.start()
        for c in conv_copies(0):
            c.start()
        x_copy(0).start()
        cp_wqkv.start()
        mx_s[...] = jnp.zeros_like(mx_s)
        ot_s[...] = jnp.zeros_like(ot_s)
        w_s[16:NPOS] = jnp.zeros((NPOS - 16, 4 * NB, 8, 128), F32)
        for h in range(H):
            qt_s[h, 16 - 16 * (h % 2):24 - 16 * (h % 2), :] = jnp.zeros((8, S), U32)
        for c in small:
            c.wait()
        par32 = jnp.concatenate([shift_ref[...].astype(F32), dvec_ref[...].astype(F32).reshape(1, D),
                                 gw_ref[...].astype(F32).reshape(1, D), jnp.zeros((2, D), F32)], axis=0)
        for dt in range(ND):
            par_s[dt] = par32[:, dt * 128:(dt + 1) * 128]

    pl.run_scoped(setup, pltpu.VMEM((4, D), BF16), pltpu.VMEM((D,), BF16), pltpu.VMEM((D,), BF16))

    def conv_tile(dt):
        for c in conv_copies(dt):
            c.wait()
        par = par_s[dt]
        fwd = fwd_ref[...]
        fwd32 = fwd.astype(F32)
        pos = pl.ds(dt * 16, 16)
        state = {"prev": None, "hist": jnp.zeros((8, 128), F32)}

        def k_part(b):
            kc = lax.dot_general(fwd, ssm_v[dt, :, b * B:(b + 1) * B], (((1,), (1,)), ((), ())),
                                 preferred_element_type=F32)
            cur = kc.reshape(16, 2, 8, 128)
            prev = state["prev"]
            if b == 0:
                cur = jnp.stack([cur[:, 0] + par[4:5], cur[:, 1]], axis=1)
                kp = cur
            else:
                re = jnp.concatenate([cur[:8, 0] - prev[:8, 1], cur[8:, 0] + prev[8:, 1]], axis=0)
                im = jnp.concatenate([cur[:8, 1] + prev[:8, 0], cur[8:, 1] - prev[8:, 0]], axis=0)
                kp = jnp.stack([re, im], axis=1)
            w_s[pos, 4 * b:4 * b + 2] = kp
            state["prev"] = cur

        def u_part(b):
            kblk = k_v[dt, b * B:(b + 1) * B, :].astype(F32)
            kx = jnp.concatenate([state["hist"], kblk], axis=0)
            state["hist"] = kblk[B - 8:B]
            ks = None
            for l in range(4):
                t = kx[8 - l:8 - l + B] * par[l:l + 1]
                ks = t if ks is None else ks + t
            kv = ks * v_v[dt, b * B:(b + 1) * B, :].astype(F32)
            w_s[pos, 4 * b + 2:4 * b + 4] = _dot(fwd32, kv).reshape(16, 2, 8, 128)

        for b in range(3):
            k_part(b)
        for b in range(NB):
            u_part(b)
            if b + 3 < NB:
                k_part(b + 3)

    qscale = (DH ** -0.5) * math.log2(math.e)

    def absmax8(a):
        a = jnp.abs(a)
        a = jnp.max(a.reshape(a.shape[0] // 8, 8, a.shape[1]), axis=0)
        r = a[:, 0:128]
        for t in range(1, a.shape[1] // 128):
            r = jnp.maximum(r, a[:, t * 128:(t + 1) * 128])
        return r

    def mac_task(p, a, z):
        yr = None
        yi = None
        for b in range(a + 1):
            kr = w_s[p + z, 4 * (a - b)]
            ki = w_s[p + z, 4 * (a - b) + 1]
            ur = w_s[p + z, 4 * b + 2]
            ui = w_s[p + z, 4 * b + 3]
            tr = kr * ur - ki * ui
            ti = kr * ui + ki * ur
            yr = tr if yr is None else yr + tr
            yi = ti if yi is None else yi + ti
        y_s[a, p, 0] = yr
        y_s[a, p, 1] = yi
        return pltpu.bitcast(_zero_bits(_u32(yr) | _u32(yi)), F32)

    def proj_phase(i):
        @pl.when(i == 0)
        def _():
            cp_wqkv.wait()

        @pl.when(i + 1 < NX)
        def _():
            x_copy(i + 1).start()

        @pl.when(i == 0)
        def _():
            for c in conv_copies(1):
                c.start()

        @pl.when(i + 2 < ND)
        def _():
            for c in conv_copies(i + 2):
                c.start()

        x_copy(i).wait()

        rows = pl.ds(pl.multiple_of(i * XC, XC), XC)
        order = [a for p in range(NB // 2) for a in (p, NB - 1 - p)]
        pbase = jnp.where(i == 0, 0, jnp.minimum(NPOS * (i - 1) + 16, 16 * ND - NPOS))
        tasks = [(f, a) for f in range(NPOS) for a in order]
        wts = [80 if rd >= 14 else 100 for rd in range((3 * ND * ND) // 4)]
        cum = np.cumsum([0] + wts)
        adds = {}
        for n, (f, a) in enumerate(tasks):
            pos = (n + 0.5) * cum[-1] / len(tasks)
            rd = int(np.searchsorted(cum, pos, side="right")) - 1
            r = int((pos - cum[rd]) / wts[rd] * (XC // 8))
            adds.setdefault(4 * rd + n % 4, {})[(r, 0)] = mac_task(pbase + f, a, i >> (10 + a))
        x = x_v[rows, :]
        cols = [None] * (3 * ND)
        for jj, j in enumerate(JORD):
            acc = None
            for k in range(ND):
                t = _dot(x[:, k * 128:(k + 1) * 128], wqkv_v[k * 128:(k + 1) * 128, j * 128:(j + 1) * 128])
                t = _add_tiles(t, adds.get(jj * ND + k))
                acc = t if acc is None else acc + t
            cols[j] = acc
        qkv = jnp.concatenate(cols, axis=1)

        kf = qkv[:, D:2 * D]
        mx_s[1] = jnp.maximum(mx_s[1], absmax8(kf))
        kf = jnp.concatenate([kf[cc * KC + 8 * e:cc * KC + 8 * e + 8]
                              for cc in range(XC // KC) for e in reversed(range(KC // 8))], axis=0)
        kk = _u32(kf.astype(BF16))
        hrows = pl.ds(pl.multiple_of(i * (XC // 2), XC // 2), XC // 2)
        lane = lax.broadcasted_iota(jnp.int32, (XC // 2, 128), 1)
        qs = qkv[:, 0:D] * qscale
        vv = qkv[:, 2 * D:3 * D]
        mx_s[0] = jnp.maximum(mx_s[0], absmax8(qs))
        mx_s[2] = jnp.maximum(mx_s[2], absmax8(vv))
        qs = qs.T
        vv = vv.T
        row8 = lax.broadcasted_iota(jnp.int32, (8, XC), 0)
        zrows = jnp.zeros((8, XC), F32)
        for h in range(H):
            w = (DH * h) // 8 * 8
            if h % 2 == 0:
                t0, off = w // 128, w % 128
                kh = kk[:, t0 * 128:(t0 + 1) * 128]
                if off:
                    kh = pltpu.roll(kh, 128 - off, 1)
                if off + 2 * DH > 128:
                    k2 = pltpu.roll(kk[:, (t0 + 1) * 128:(t0 + 2) * 128], 128 - off, 1)
                    kh = jnp.where(lane < 128 - off, kh, k2)
                kk_s[h // 2, hrows, :] = kh
            if h == 0:
                nvx = NVB // NX
                src = jnp.concatenate([kh[c * KC // 2 + 8 * e:c * KC // 2 + 8 * e + 8] for c, e in VBLK[:nvx]], axis=0)
                for d in range(DH):
                    col = _bf(jnp.broadcast_to(src[:, d:d + 1], src.shape)).astype(F32)
                    kb0[0, pl.ds(i * nvx, nvx), d] = col.reshape(nvx, 16, 128)
            qw = qs[w:w + 24, :]
            vw = vv[w:w + 24, :]
            qf_s[h, :, rows] = qw
            if h % 2 == 0:
                qparts = [qw[0:16], jnp.where(row8 < 4, qw[16:24], 0.0)]
                vparts = [vw[0:16], jnp.where(row8 == 4, 1.0, vw[16:24])]
            else:
                qparts = [jnp.where(row8 >= 4, qw[0:8], 0.0), qw[8:24]]
                vparts = [jnp.where(row8 == 0, 1.0, vw[0:8]), vw[8:24]]
            qt = _u32(jnp.concatenate(qparts + [zrows], axis=0).astype(BF16))
            qt_s[h, 8 * (h % 2):8 * (h % 2) + 16, rows] = qt
            vt_s[h, :, rows] = jnp.concatenate(vparts, axis=0)

    def pre_phase(t, carry):
        u = jnp.where(t == 1, 2, jnp.where(t == 2, 1, t))
        is_conv = (u == 0) | ((u & 1) == 1)
        lax.cond(is_conv, lambda: conv_tile((u + 1) >> 1), lambda: proj_phase((u - 2) >> 1))
        return carry

    lax.fori_loop(0, ND + NX, pre_phase, 0)
    cp_wo.start()

    def unrev(s):
        return jnp.concatenate([s[8 * e:8 * e + 8] for e in reversed(range(s.shape[0] // 8))], axis=0)

    def finish(acc, hp, par, q2):
        if isinstance(par, int):
            den = acc[20:21, :] if par == 0 else acc[0:1, :]
        else:
            den = jnp.where(par == 0, acc[20:21, :], acc[0:1, :])
        o = acc * pl.reciprocal(den, approx=False)
        w = pl.multiple_of(hp * 40 + par * 16, 8)
        row = lax.broadcasted_iota(jnp.int32, (24, TQ), 0)
        msk = (row >= 4 * par) & (row < 4 * par + DH)
        pltpu.store(ot_s.at[pl.ds(w, 24), q2 * TQ:(q2 + 1) * TQ], o, mask=msk)

    def qk(hp, h, kd, qi, *ranges):
        lhs = jnp.concatenate([kk_s[hp, lo // 2:hi // 2, :] for lo, hi in ranges if hi > lo], axis=0)
        return _dot(_bf(lhs)[:, 0:kd], _bf(qt_s[h, 0:kd // 2, qi * TQ:(qi + 1) * TQ]))

    def pv(h, c, p, acc):
        o = _dot(vt_s[h, :, c * KC:(c + 1) * KC], p)
        return o if acc is None else acc + o

    def slow_path():
        sb = [s0, s1]
        mb = [m0, m1]
        s1[...] = jnp.zeros_like(s1)
        m1[...] = jnp.zeros_like(m1)

        def fused(h1, q1, h2, q2, z1, z2):
            sA, mA = sb[q1 % 2], mb[q1 % 2]
            sB, mB = sb[q2 % 2], mb[q2 % 2]
            mcur = mB[0:1, :]
            m = None
            acc = None
            for c in range(NC):
                if h1 is not None:
                    s = qk(h1 >> 1, h1, 48, q1, (c * KC, (c + 1) * KC))
                    sA[z1, c * KC:(c + 1) * KC, :] = unrev(s)
                    mc = jnp.max(s.reshape(KC // 8, 8, TQ), axis=0)
                    m = mc if m is None else jnp.maximum(m, mc)
                p = jnp.exp2(sB[z2, c * KC:(c + 1) * KC, :] - mcur)
                acc = pv(h2, c, p, acc)
            if h1 is not None:
                mA[0:1, :] = jnp.max(m, axis=0, keepdims=True)
            finish(acc, h2 >> 1, h2 & 1, q2)

        def body(h, carry):
            z1 = h >> 10
            z2 = h >> 11
            fused(h, 0, jnp.maximum(h - 1, 0), NQ - 1, z1, z2)
            for qi in range(1, NQ):
                fused(h, qi, h, qi - 1, z1, z2)
            return carry

        lax.fori_loop(0, H, body, 0)
        fused(None, 0, jnp.int32(H - 1), NQ - 1, 0, 0)

    def fast_path():
        def make_kb(hp, par, d, gate):
            z = _zero_bits(_u32(gate))
            kk = jnp.concatenate([kk_s[hp, c * KC // 2 + 8 * e:c * KC // 2 + 8 * e + 8, :] | z for c, e in VBLK],
                                 axis=0)
            col = _bf(jnp.broadcast_to(kk[:, DH * par + d:DH * par + d + 1], kk.shape)).astype(F32)
            kb_s[par][0, :, d] = col.reshape(NVB, 16, 128)

        def vpu_chain(i, par, qi, c, e, t):
            v = VBLK.index((c, e))
            hq = 2 * i + par + (i >> (8 + v))
            zz = i >> (10 + qi * NT + t)
            acc = None
            for d in range(DH):
                qb = jnp.broadcast_to(
                    qf_s[hq, 4 * par + d:4 * par + d + 1, qi * TQ + t * 128:qi * TQ + (t + 1) * 128], (8, 128))
                pr = kb_s[par][zz, v, d] * jnp.concatenate([qb, qb], axis=0)
                acc = pr if acc is None else acc + pr
            return acc

        def body(i, carry):
            steps = [(par, qi, c) for par in range(2) for qi in range(NQ) for c in range(NC)]
            nv = [NV[c] if n >= 1 else 0 for n, (par, qi, c) in enumerate(steps)]
            queue = [(n, e, t) for n in range(len(steps)) for e in range(nv[n]) for t in range(NT)]
            quota = NVB * NT // NC
            sv = {}
            early = None
            pend = None
            acc = None

            def drain(acc):
                par, qi, c, p = pend
                acc = pv(2 * i + par, c, p, acc)
                if c == NC - 1:
                    finish(acc, i, par, qi)
                    acc = acc * 0.0
                return acc

            for step, (par, qi, c) in enumerate(steps):
                lo = c * KC + 16 * nv[step] + (16 if c > 0 else 0)
                lo2 = (c + 1) * KC + 16 * nv[step + 1] if c + 1 < NC else 0
                n2 = 16 if c + 1 < NC else 0
                s = qk(i, 2 * i + par, 48 if par else 32, qi, (lo, (c + 1) * KC), (lo2, lo2 + n2))
                gate = s[0:8, 0:128]
                todo = []
                while queue and (queue[0][0] <= step + 1 or
                                 (len(todo) < quota and steps[queue[0][0]][0] == par)):
                    todo.append(queue.pop(0))
                adds = {}
                for k, (n, e, t) in enumerate(todo):
                    a = vpu_chain(i, steps[n][0], steps[n][1], steps[n][2], e, t)
                    sv[(n, e, t)] = a
                    adds[((k * (s.shape[0] // 8)) // len(todo), NT - 1)] = (a[0:8] + a[8:16]) * 0.0
                s = _add_tiles(s, adds)
                x = [jnp.concatenate([sv.pop((step, e, t)) for t in range(NT)], axis=1) for e in range(nv[step])]
                if early is not None:
                    x.append(early)
                early = None
                if n2:
                    early = s[s.shape[0] - n2:]
                    s = s[:s.shape[0] - n2]
                p = jnp.exp2(unrev(jnp.concatenate(x + [s], axis=0)))
                if pend is not None:
                    acc = drain(acc)
                pend = (par, qi, c, p)
                n = qi * NC + c
                if n % 3 == 1 and n // 3 < DH:
                    make_kb(jnp.minimum(i + 1, H // 2 - 1) if par else i, 1 - par, n // 3, gate)
            drain(acc)
            return carry

        lax.fori_loop(0, H // 2, body, 0)

    qmax = jnp.max(mx_s[0])
    kmax = jnp.max(mx_s[1])
    vmax = jnp.max(mx_s[2])
    safe = (qmax * kmax * DH <= 80.0) & (vmax <= 2.0 ** 30) & (vmax >= 2.0 ** -30)
    lax.cond(safe, fast_path, slow_path)

    cp_wo.wait()

    def out_copy(i, nb):
        rows = pl.ds(pl.multiple_of(i * EB * B, B), nb * B)
        return pltpu.make_async_copy(out_v.at[rows, :], out_hbm.at[0, rows, :], sem_o.at[i])

    def epilogue(i, nb):
        rows = pl.ds(pl.multiple_of(i * EB * B, B), nb * B)
        inv = inv_ref[...].astype(F32)
        ys = []
        for bb in range(nb):
            yf = jnp.concatenate([y_s[i * EB + bb, dt * 16:(dt + 1) * 16].reshape(2 * B, 128) for dt in range(ND)], axis=1)
            ys.append(_dot(inv, yf))
        y = jnp.concatenate(ys, axis=0)
        o = ot_s[:, rows].T.astype(BF16)
        adds = {}
        tiles = [(a, b) for a in range(nb) for b in range(ND)]
        for n, (a, b) in enumerate(tiles):
            z = _zero_bits(_u32(o[a * 128 + 112:a * 128 + 128, b * 128:(b + 1) * 128]))
            pos = (2 * len(tiles) + 10 * n) // 20
            adds[((pos // ND) * 16 + n % 16, pos % ND)] = pltpu.bitcast(z, F32)
        y = _add_tiles(y, adds)
        bres = _dot(o, wo_v[...])
        x = x_v[rows, :].astype(F32)
        logit = jnp.sum(x * jnp.concatenate([par_s[dt, 5:6, :] for dt in range(ND)], axis=1), axis=-1, keepdims=True)
        gate = jax.nn.sigmoid(logit)
        out_v[rows, :] = (bres + gate * (x * y - bres)).astype(BF16)
        out_copy(i, nb).start()

    def epilogue_body(i, carry):
        epilogue(i, EB)
        return carry

    ne = NB // EB
    lax.fori_loop(0, ne, epilogue_body, 0)
    epilogue(ne, NB % EB)
    for i in range(ne):
        out_copy(i, EB).wait()
    out_copy(ne, NB % EB).wait()


@jax.jit
def pallas_gated_mix__ssm_conv_h3__mha_block__prompt_kernel(
    A_q: jax.Array,
    A_k: jax.Array,
    A_v: jax.Array,
    A_shift_k: jax.Array,
    A_ssm_k: jax.Array,
    A_ssm_D: jax.Array,
    B_x: jax.Array,
    B_wqkv: jax.Array,
    B_wo: jax.Array,
    gate_w: jax.Array,
):
    del B_x
    fwd, inv = _dft_consts()
    any_spec = pl.BlockSpec(memory_space=pl.ANY)
    scratch = [
        pltpu.VMEM((4, 8, 128), F32),
        pltpu.VMEM((2 * B, B), BF16),
        pltpu.VMEM((B, 2 * B), BF16),
        pltpu.VMEM((S, D), BF16),
        pltpu.VMEM((ND, S, 128), BF16),
        pltpu.VMEM((ND, S, 128), BF16),
        pltpu.VMEM((ND, 128, S), BF16),
        pltpu.VMEM((D, 3 * D), BF16),
        pltpu.VMEM((D, D), BF16),
        pltpu.VMEM((S, D), BF16),
        pltpu.VMEM((H, 24, S), U32),
        pltpu.VMEM((H // 2, S // 2, 128), U32),
        pltpu.VMEM((H, 24, S), F32),
        pltpu.VMEM((1, S, TQ), F32),
        pltpu.VMEM((1, S, TQ), F32),
        pltpu.VMEM((8, TQ), F32),
        pltpu.VMEM((8, TQ), F32),
        pltpu.VMEM((D, S), F32),
        pltpu.VMEM((16 * ND, 4 * NB, 8, 128), F32),
        pltpu.VMEM((8, 8, 128), F32),
        pltpu.VMEM((NB, 16 * ND, 2, 8, 128), F32),
        pltpu.VMEM((H, 24, S), F32),
        pltpu.VMEM((1, NVB, DH, 16, 128), F32),
        pltpu.VMEM((1, NVB, DH, 16, 128), F32),
        pltpu.SemaphoreType.DMA((2,)),
        pltpu.SemaphoreType.DMA((NX,)),
        pltpu.SemaphoreType.DMA((3 * ND,)),
        pltpu.SemaphoreType.DMA((NB // EB + 1,)),
        pltpu.SemaphoreType.DMA((5,)),
    ]
    return pl.pallas_call(
        _kernel,
        out_shape=jax.ShapeDtypeStruct((1, S, D), BF16),
        in_specs=[any_spec] * 11,
        out_specs=any_spec,
        scratch_shapes=scratch,
        compiler_params=pltpu.CompilerParams(vmem_limit_bytes=120 * 2 ** 20, disable_bounds_checks=True,
                                             internal_scratch_in_bytes=3 * 16384),
    )(A_q, A_k, A_v, A_ssm_k, B_wqkv, B_wo,
      A_shift_k.T, A_ssm_D, gate_w,
      jnp.asarray(fwd, BF16), jnp.asarray(inv, BF16))
```

```python
import math

import numpy as np
import jax
import jax.numpy as jnp
from jax import lax
import jax.experimental.pallas as pl
import jax.experimental.pallas.tpu as pltpu

S = 2048
D = 640
H = 32
DH = 20
ND = D // 128
TQ = 512
NQ = S // TQ
NT = TQ // 128
KC = 128
NC = S // KC
B = 128
NB = S // B
XC = 512
NX = S // XC
NPOS = 22
EB = 5
NV = [2, 1, 1, 1] * (NC // 4)
NVB = sum(NV)
VBLK = [(c, e) for c in range(NC) for e in range(NV[c])]
JORD = [0, 1, 2, 3, 4, 5, 10, 11, 12, 13, 14, 6, 7, 8, 9]

F32 = jnp.float32
BF16 = jnp.bfloat16
U32 = jnp.uint32


def _dft_consts():
    r = np.arange(2 * B)
    t, part, i = r // 16, (r // 8) % 2, r % 8
    f = np.where(t < 8, 2 * (8 * t + i), 2 * (8 * (t - 8) + i) + 1)
    theta = np.pi * (2 * f + 1) / (2 * B)
    ang = theta[:, None] * np.arange(B)[None, :]
    fwd = np.where(part[:, None] == 0, np.cos(ang), -np.sin(ang))
    inv = fwd.T / B
    return fwd.astype(np.float32), inv.astype(np.float32)


def _bf(x):
    return pltpu.bitcast(x, BF16)


def _u32(x):
    return pltpu.bitcast(x, U32)


def _dot(a, b):
    return jnp.dot(a, b, precision=lax.Precision.DEFAULT, preferred_element_type=F32)


def _zero_bits(u):
    return lax.shift_right_logical(lax.shift_right_logical(u, U32(31)), U32(1))


def _add_tiles(s, adds):
    if not adds:
        return s
    rows = []
    done = 0
    for r in sorted({r for r, _ in adds}):
        if 8 * r > done:
            rows.append(s[done:8 * r])
        row = s[8 * r:8 * r + 8]
        parts = []
        cdone = 0
        for t in sorted(t for rr, t in adds if rr == r):
            if 128 * t > cdone:
                parts.append(row[:, cdone:128 * t])
            parts.append(row[:, 128 * t:128 * (t + 1)] + adds[(r, t)])
            cdone = 128 * (t + 1)
        if cdone < s.shape[1]:
            parts.append(row[:, cdone:])
        rows.append(jnp.concatenate(parts, axis=1))
        done = 8 * r + 8
    if done < s.shape[0]:
        rows.append(s[done:])
    return jnp.concatenate(rows, axis=0)


def _kernel(x_hbm, k_hbm, v_hbm, ssm_hbm, wqkv_hbm, wo_hbm,
            shift_hbm, dvec_hbm, gw_hbm, fwd_hbm, inv_hbm,
            out_hbm,
            mx_s, fwd_ref, inv_ref, x_v, k_v, v_v, ssm_v, wqkv_v, wo_v, out_v,
            qt_s, kk_s, vt_s, s0, s1, m0, m1, ot_s,
            w_s, par_s, y_s, qf_s, kb0, kb1, ks_s,
            sem_w, sem_x, sem_c, sem_o, sem_s):
    kb_s = (kb0, kb1)
    cp_wqkv = pltpu.make_async_copy(wqkv_hbm, wqkv_v, sem_w.at[0])
    cp_wo = pltpu.make_async_copy(wo_hbm, wo_v, sem_w.at[1])

    def x_copy(i):
        rows = pl.ds(pl.multiple_of(i * XC, XC), XC)
        return pltpu.make_async_copy(x_hbm.at[0, rows, :], x_v.at[rows, :], sem_x.at[i])

    def conv_copies(dt):
        ln = pl.ds(pl.multiple_of(dt * 128, 128), 128)
        return [
            pltpu.make_async_copy(ssm_hbm.at[ln, :], ssm_v.at[dt], sem_c.at[3 * dt]),
            pltpu.make_async_copy(k_hbm.at[0, :, ln], k_v.at[dt], sem_c.at[3 * dt + 1]),
            pltpu.make_async_copy(v_hbm.at[0, :, ln], v_v.at[dt], sem_c.at[3 * dt + 2]),
        ]

    def setup(shift_ref, dvec_ref, gw_ref):
        small = [pltpu.make_async_copy(src, dst, sem_s.at[n]) for n, (src, dst) in enumerate(
            [(shift_hbm, shift_ref), (dvec_hbm, dvec_ref), (gw_hbm, gw_ref), (fwd_hbm, fwd_ref), (inv_hbm, inv_ref)])]
        for c in small:
            c.start()
        for c in conv_copies(0):
            c.start()
        x_copy(0).start()
        cp_wqkv.start()
        mx_s[...] = jnp.zeros_like(mx_s)
        ot_s[...] = jnp.zeros_like(ot_s)
        w_s[16:NPOS] = jnp.zeros((NPOS - 16, 4 * NB, 8, 128), F32)
        for h in range(H):
            qt_s[h, 16 - 16 * (h % 2):24 - 16 * (h % 2), :] = jnp.zeros((8, S), U32)
        for c in small:
            c.wait()
        par32 = jnp.concatenate([shift_ref[...].astype(F32), dvec_ref[...].astype(F32).reshape(1, D),
                                 gw_ref[...].astype(F32).reshape(1, D), jnp.zeros((2, D), F32)], axis=0)
        for dt in range(ND):
            par_s[dt] = par32[:, dt * 128:(dt + 1) * 128]

    pl.run_scoped(setup, pltpu.VMEM((4, D), BF16), pltpu.VMEM((D,), BF16), pltpu.VMEM((D,), BF16))

    def conv_tile(dt):
        for c in conv_copies(dt):
            c.wait()
        par = par_s[dt]
        fwd = fwd_ref[...]
        fwd32 = fwd.astype(F32)
        pos = pl.ds(dt * 16, 16)
        state = {"prev": None, "hist": jnp.zeros((8, 128), F32)}

        def k_part(b):
            kc = lax.dot_general(fwd, ssm_v[dt, :, b * B:(b + 1) * B], (((1,), (1,)), ((), ())),
                                 preferred_element_type=F32)
            cur = kc.reshape(16, 2, 8, 128)
            prev = state["prev"]
            if b == 0:
                cur = jnp.stack([cur[:, 0] + par[4:5], cur[:, 1]], axis=1)
                kp = cur
            else:
                re = jnp.concatenate([cur[:8, 0] - prev[:8, 1], cur[8:, 0] + prev[8:, 1]], axis=0)
                im = jnp.concatenate([cur[:8, 1] + prev[:8, 0], cur[8:, 1] - prev[8:, 0]], axis=0)
                kp = jnp.stack([re, im], axis=1)
            w_s[pos, 4 * b:4 * b + 2] = kp
            state["prev"] = cur

        def u_part(b):
            kblk = k_v[dt, b * B:(b + 1) * B, :].astype(F32)
            kx = jnp.concatenate([state["hist"], kblk], axis=0)
            state["hist"] = kblk[B - 8:B]
            ks = None
            for l in range(4):
                t = kx[8 - l:8 - l + B] * par[l:l + 1]
                ks = t if ks is None else ks + t
            kv = ks * v_v[dt, b * B:(b + 1) * B, :].astype(F32)
            w_s[pos, 4 * b + 2:4 * b + 4] = _dot(fwd32, kv).reshape(16, 2, 8, 128)

        for b in range(3):
            k_part(b)
        for b in range(NB):
            u_part(b)
            if b + 3 < NB:
                k_part(b + 3)

    qscale = (DH ** -0.5) * math.log2(math.e)

    def absmax8(a):
        a = jnp.abs(a)
        a = jnp.max(a.reshape(a.shape[0] // 8, 8, a.shape[1]), axis=0)
        r = a[:, 0:128]
        for t in range(1, a.shape[1] // 128):
            r = jnp.maximum(r, a[:, t * 128:(t + 1) * 128])
        return r

    def mac_task(p, a, z):
        yr = None
        yi = None
        for b in range(a + 1):
            kr = w_s[p + z, 4 * (a - b)]
            ki = w_s[p + z, 4 * (a - b) + 1]
            ur = w_s[p + z, 4 * b + 2]
            ui = w_s[p + z, 4 * b + 3]
            tr = kr * ur - ki * ui
            ti = kr * ui + ki * ur
            yr = tr if yr is None else yr + tr
            yi = ti if yi is None else yi + ti
        y_s[a, p, 0] = yr
        y_s[a, p, 1] = yi
        return pltpu.bitcast(_zero_bits(_u32(yr) | _u32(yi)), F32)

    def proj_phase(i):
        @pl.when(i == 0)
        def _():
            cp_wqkv.wait()

        @pl.when(i + 1 < NX)
        def _():
            x_copy(i + 1).start()

        @pl.when(i == 0)
        def _():
            for c in conv_copies(1):
                c.start()

        @pl.when(i + 2 < ND)
        def _():
            for c in conv_copies(i + 2):
                c.start()

        x_copy(i).wait()

        rows = pl.ds(pl.multiple_of(i * XC, XC), XC)
        order = [a for p in range(NB // 2) for a in (p, NB - 1 - p)]
        pbase = jnp.where(i == 0, 0, jnp.minimum(NPOS * (i - 1) + 16, 16 * ND - NPOS))
        tasks = [(f, a) for f in range(NPOS) for a in order]
        wts = [80 if rd >= 14 else 100 for rd in range((3 * ND * ND) // 4)]
        cum = np.cumsum([0] + wts)
        adds = {}
        for n, (f, a) in enumerate(tasks):
            pos = (n + 0.5) * cum[-1] / len(tasks)
            rd = int(np.searchsorted(cum, pos, side="right")) - 1
            r = int((pos - cum[rd]) / wts[rd] * (XC // 8))
            adds.setdefault(4 * rd + n % 4, {})[(r, 0)] = mac_task(pbase + f, a, i >> (10 + a))
        x = x_v[rows, :]
        cols = [None] * (3 * ND)
        for jj, j in enumerate(JORD):
            acc = None
            for k in range(ND):
                t = _dot(x[:, k * 128:(k + 1) * 128], wqkv_v[k * 128:(k + 1) * 128, j * 128:(j + 1) * 128])
                t = _add_tiles(t, adds.get(jj * ND + k))
                acc = t if acc is None else acc + t
            cols[j] = acc
        qkv = jnp.concatenate(cols, axis=1)

        kf = qkv[:, D:2 * D]
        mx_s[1] = jnp.maximum(mx_s[1], absmax8(kf))
        kf = jnp.concatenate([kf[cc * KC + 8 * e:cc * KC + 8 * e + 8]
                              for cc in range(XC // KC) for e in reversed(range(KC // 8))], axis=0)
        kk = _u32(kf.astype(BF16))
        hrows = pl.ds(pl.multiple_of(i * (XC // 2), XC // 2), XC // 2)
        lane = lax.broadcasted_iota(jnp.int32, (XC // 2, 128), 1)
        qs = qkv[:, 0:D] * qscale
        vv = qkv[:, 2 * D:3 * D]
        mx_s[0] = jnp.maximum(mx_s[0], absmax8(qs))
        mx_s[2] = jnp.maximum(mx_s[2], absmax8(vv))
        qs = qs.T
        vv = vv.T
        row8 = lax.broadcasted_iota(jnp.int32, (8, XC), 0)
        zrows = jnp.zeros((8, XC), F32)
        for h in range(H):
            w = (DH * h) // 8 * 8
            if h % 2 == 0:
                t0, off = w // 128, w % 128
                kh = kk[:, t0 * 128:(t0 + 1) * 128]
                if off:
                    kh = pltpu.roll(kh, 128 - off, 1)
                if off + 2 * DH > 128:
                    k2 = pltpu.roll(kk[:, (t0 + 1) * 128:(t0 + 2) * 128], 128 - off, 1)
                    kh = jnp.where(lane < 128 - off, kh, k2)
                kk_s[h // 2, hrows, :] = kh
            if h == 0:
                nvx = NVB // NX
                src = jnp.concatenate([kh[c * KC // 2 + 8 * e:c * KC // 2 + 8 * e + 8] for c, e in VBLK[:nvx]], axis=0)
                for d in range(DH):
                    col = _bf(jnp.broadcast_to(src[:, d:d + 1], src.shape)).astype(F32)
                    kb0[0, pl.ds(i * nvx, nvx), d] = col.reshape(nvx, 16, 128)
            qw = qs[w:w + 24, :]
            vw = vv[w:w + 24, :]
            qf_s[h, :, rows] = qw
            if h % 2 == 0:
                qparts = [qw[0:16], jnp.where(row8 < 4, qw[16:24], 0.0)]
                vparts = [vw[0:16], jnp.where(row8 == 4, 1.0, vw[16:24])]
            else:
                qparts = [jnp.where(row8 >= 4, qw[0:8], 0.0), qw[8:24]]
                vparts = [jnp.where(row8 == 0, 1.0, vw[0:8]), vw[8:24]]
            qt = _u32(jnp.concatenate(qparts + [zrows], axis=0).astype(BF16))
            qt_s[h, 8 * (h % 2):8 * (h % 2) + 16, rows] = qt
            vt_s[h, :, rows] = jnp.concatenate(vparts, axis=0)

    def pre_phase(t, carry):
        u = jnp.where(t == 1, 2, jnp.where(t == 2, 1, t))
        is_conv = (u == 0) | ((u & 1) == 1)
        lax.cond(is_conv, lambda: conv_tile((u + 1) >> 1), lambda: proj_phase((u - 2) >> 1))
        return carry

    lax.fori_loop(0, ND + NX, pre_phase, 0)
    cp_wo.start()

    def unrev(s):
        return jnp.concatenate([s[8 * e:8 * e + 8] for e in reversed(range(s.shape[0] // 8))], axis=0)

    def finish(acc, hp, par, q2):
        if isinstance(par, int):
            den = acc[20:21, :] if par == 0 else acc[0:1, :]
        else:
            den = jnp.where(par == 0, acc[20:21, :], acc[0:1, :])
        o = acc * pl.reciprocal(den, approx=False)
        w = pl.multiple_of(hp * 40 + par * 16, 8)
        row = lax.broadcasted_iota(jnp.int32, (24, TQ), 0)
        msk = (row >= 4 * par) & (row < 4 * par + DH)
        pltpu.store(ot_s.at[pl.ds(w, 24), q2 * TQ:(q2 + 1) * TQ], o, mask=msk)

    def qk(hp, h, kd, qi, *ranges):
        lhs = jnp.concatenate([kk_s[hp, lo // 2:hi // 2, :] for lo, hi in ranges if hi > lo], axis=0)
        return _dot(_bf(lhs)[:, 0:kd], _bf(qt_s[h, 0:kd // 2, qi * TQ:(qi + 1) * TQ]))

    def pv(h, c, p, acc):
        o = _dot(vt_s[h, :, c * KC:(c + 1) * KC], p)
        return o if acc is None else acc + o

    def slow_path():
        sb = [s0, s1]
        mb = [m0, m1]
        s1[...] = jnp.zeros_like(s1)
        m1[...] = jnp.zeros_like(m1)

        def fused(h1, q1, h2, q2, z1, z2):
            sA, mA = sb[q1 % 2], mb[q1 % 2]
            sB, mB = sb[q2 % 2], mb[q2 % 2]
            mcur = mB[0:1, :]
            m = None
            acc = None
            for c in range(NC):
                if h1 is not None:
                    s = qk(h1 >> 1, h1, 48, q1, (c * KC, (c + 1) * KC))
                    sA[z1, c * KC:(c + 1) * KC, :] = unrev(s)
                    mc = jnp.max(s.reshape(KC // 8, 8, TQ), axis=0)
                    m = mc if m is None else jnp.maximum(m, mc)
                p = jnp.exp2(sB[z2, c * KC:(c + 1) * KC, :] - mcur)
                acc = pv(h2, c, p, acc)
            if h1 is not None:
                mA[0:1, :] = jnp.max(m, axis=0, keepdims=True)
            finish(acc, h2 >> 1, h2 & 1, q2)

        def body(h, carry):
            z1 = h >> 10
            z2 = h >> 11
            fused(h, 0, jnp.maximum(h - 1, 0), NQ - 1, z1, z2)
            for qi in range(1, NQ):
                fused(h, qi, h, qi - 1, z1, z2)
            return carry

        lax.fori_loop(0, H, body, 0)
        fused(None, 0, jnp.int32(H - 1), NQ - 1, 0, 0)

    def fast_path():
        def stage_k(i, hp, gate):
            z = _zero_bits(_u32(gate))
            kk = jnp.concatenate([kk_s[hp, c * KC // 2 + 8 * e:c * KC // 2 + 8 * e + 8, :] | z for c, e in VBLK],
                                 axis=0)
            ks_s[i >> 9, 0:16 * NVB, :] = _bf(kk).astype(F32)

        def make_kb(i, par, d, v0, v1, gate):
            ks_s[i >> 8, 16 * NVB:16 * NVB + 8, :] = gate
            src = ks_s[i >> (10 + d), 16 * v0:16 * v1, :]
            col = jnp.broadcast_to(src[:, DH * par + d:DH * par + d + 1], src.shape)
            kb_s[par][0, v0:v1, d] = col.reshape(v1 - v0, 16, 128)

        def vpu_chain(i, par, qi, c, e, t):
            v = VBLK.index((c, e))
            hq = 2 * i + par + (i >> (8 + v))
            zz = i >> (10 + qi * NT + t)
            acc = None
            for d in range(DH):
                qb = jnp.broadcast_to(
                    qf_s[hq, 4 * par + d:4 * par + d + 1, qi * TQ + t * 128:qi * TQ + (t + 1) * 128], (8, 128))
                pr = kb_s[par][zz, v, d] * jnp.concatenate([qb, qb], axis=0)
                acc = pr if acc is None else acc + pr
            return acc

        def body(i, carry):
            steps = [(par, qi, c) for par in range(2) for qi in range(NQ) for c in range(NC)]
            nv = [NV[c] if n >= 1 else 0 for n, (par, qi, c) in enumerate(steps)]
            queue = [(n, e, t) for n in range(len(steps)) for e in range(nv[n]) for t in range(NT)]
            quota = NVB * NT // NC
            sv = {}
            early = None
            pend = []
            acc = None

            def drain(acc):
                par, qi, c, p = pend.pop(0)
                acc = pv(2 * i + par, c, p, acc)
                if c == NC - 1:
                    finish(acc, i, par, qi)
                    acc = acc * 0.0
                return acc

            for step, (par, qi, c) in enumerate(steps):
                lo = c * KC + 16 * nv[step] + (16 if c > 0 else 0)
                lo2 = (c + 1) * KC + 16 * nv[step + 1] if c + 1 < NC else 0
                n2 = 16 if c + 1 < NC else 0
                s = qk(i, 2 * i + par, 48 if par else 32, qi, (lo, (c + 1) * KC), (lo2, lo2 + n2))
                gate = s[0:8, 0:128]
                todo = []
                while queue and (queue[0][0] <= step + 1 or
                                 (len(todo) < quota and steps[queue[0][0]][0] == par)):
                    todo.append(queue.pop(0))
                adds = {}
                for k, (n, e, t) in enumerate(todo):
                    a = vpu_chain(i, steps[n][0], steps[n][1], steps[n][2], e, t)
                    sv[(n, e, t)] = a
                    adds[((k * (s.shape[0] // 8)) // len(todo), NT - 1)] = (a[0:8] + a[8:16]) * 0.0
                s = _add_tiles(s, adds)
                x = [jnp.concatenate([sv.pop((step, e, t)) for t in range(NT)], axis=1) for e in range(nv[step])]
                if early is not None:
                    x.append(early)
                early = None
                if n2:
                    early = s[s.shape[0] - n2:]
                    s = s[:s.shape[0] - n2]
                p = jnp.exp2(unrev(jnp.concatenate(x + [s], axis=0)))
                if pend and step < len(steps) - 4:
                    acc = drain(acc)
                pend.append((par, qi, c, p))
                n = qi * NC + c
                if n == 0 and par == 1:
                    stage_k(i, jnp.minimum(i + 1, H // 2 - 1), gate)
                if n % 3 > 0 and n // 3 < DH:
                    part = n % 3 - 1
                    make_kb(i, 1 - par, n // 3, part * NVB // 2, (part + 1) * NVB // 2, gate)
            while pend:
                acc = drain(acc)
            return carry

        stage_k(jnp.int32(0), 0, jnp.zeros((8, 128), F32))
        lax.fori_loop(0, H // 2, body, 0)

    qmax = jnp.max(mx_s[0])
    kmax = jnp.max(mx_s[1])
    vmax = jnp.max(mx_s[2])
    safe = (qmax * kmax * DH <= 80.0) & (vmax <= 2.0 ** 30) & (vmax >= 2.0 ** -30)
    lax.cond(safe, fast_path, slow_path)

    cp_wo.wait()

    def out_copy(i, nb):
        rows = pl.ds(pl.multiple_of(i * EB * B, B), nb * B)
        return pltpu.make_async_copy(out_v.at[rows, :], out_hbm.at[0, rows, :], sem_o.at[i])

    def epilogue(i, nb):
        rows = pl.ds(pl.multiple_of(i * EB * B, B), nb * B)
        inv = inv_ref[...].astype(F32)
        ys = []
        for bb in range(nb):
            yf = jnp.concatenate([y_s[i * EB + bb, dt * 16:(dt + 1) * 16].reshape(2 * B, 128) for dt in range(ND)], axis=1)
            ys.append(_dot(inv, yf))
        y = jnp.concatenate(ys, axis=0)
        o = ot_s[:, rows].T.astype(BF16)
        adds = {}
        tiles = [(a, b) for a in range(nb) for b in range(ND)]
        for n, (a, b) in enumerate(tiles):
            z = _zero_bits(_u32(o[a * 128 + 112:a * 128 + 128, b * 128:(b + 1) * 128]))
            pos = (2 * len(tiles) + 10 * n) // 20
            adds[((pos // ND) * 16 + n % 16, pos % ND)] = pltpu.bitcast(z, F32)
        y = _add_tiles(y, adds)
        bres = _dot(o, wo_v[...])
        x = x_v[rows, :].astype(F32)
        logit = jnp.sum(x * jnp.concatenate([par_s[dt, 5:6, :] for dt in range(ND)], axis=1), axis=-1, keepdims=True)
        gate = jax.nn.sigmoid(logit)
        out_v[rows, :] = (bres + gate * (x * y - bres)).astype(BF16)
        out_copy(i, nb).start()

    def epilogue_body(i, carry):
        epilogue(i, EB)
        return carry

    ne = NB // EB
    lax.fori_loop(0, ne, epilogue_body, 0)
    epilogue(ne, NB % EB)
    for i in range(ne):
        out_copy(i, EB).wait()
    out_copy(ne, NB % EB).wait()


@jax.jit
def pallas_gated_mix__ssm_conv_h3__mha_block__prompt_kernel(
    A_q: jax.Array,
    A_k: jax.Array,
    A_v: jax.Array,
    A_shift_k: jax.Array,
    A_ssm_k: jax.Array,
    A_ssm_D: jax.Array,
    B_x: jax.Array,
    B_wqkv: jax.Array,
    B_wo: jax.Array,
    gate_w: jax.Array,
):
    del B_x
    fwd, inv = _dft_consts()
    any_spec = pl.BlockSpec(memory_space=pl.ANY)
    scratch = [
        pltpu.VMEM((4, 8, 128), F32),
        pltpu.VMEM((2 * B, B), BF16),
        pltpu.VMEM((B, 2 * B), BF16),
        pltpu.VMEM((S, D), BF16),
        pltpu.VMEM((ND, S, 128), BF16),
        pltpu.VMEM((ND, S, 128), BF16),
        pltpu.VMEM((ND, 128, S), BF16),
        pltpu.VMEM((D, 3 * D), BF16),
        pltpu.VMEM((D, D), BF16),
        pltpu.VMEM((S, D), BF16),
        pltpu.VMEM((H, 24, S), U32),
        pltpu.VMEM((H // 2, S // 2, 128), U32),
        pltpu.VMEM((H, 24, S), F32),
        pltpu.VMEM((1, S, TQ), F32),
        pltpu.VMEM((1, S, TQ), F32),
        pltpu.VMEM((8, TQ), F32),
        pltpu.VMEM((8, TQ), F32),
        pltpu.VMEM((D, S), F32),
        pltpu.VMEM((16 * ND, 4 * NB, 8, 128), F32),
        pltpu.VMEM((8, 8, 128), F32),
        pltpu.VMEM((NB, 16 * ND, 2, 8, 128), F32),
        pltpu.VMEM((H, 24, S), F32),
        pltpu.VMEM((1, NVB, DH, 16, 128), F32),
        pltpu.VMEM((1, NVB, DH, 16, 128), F32),
        pltpu.VMEM((1, 16 * NVB + 32, 128), F32),
        pltpu.SemaphoreType.DMA((2,)),
        pltpu.SemaphoreType.DMA((NX,)),
        pltpu.SemaphoreType.DMA((3 * ND,)),
        pltpu.SemaphoreType.DMA((NB // EB + 1,)),
        pltpu.SemaphoreType.DMA((5,)),
    ]
    return pl.pallas_call(
        _kernel,
        out_shape=jax.ShapeDtypeStruct((1, S, D), BF16),
        in_specs=[any_spec] * 11,
        out_specs=any_spec,
        scratch_shapes=scratch,
        compiler_params=pltpu.CompilerParams(vmem_limit_bytes=120 * 2 ** 20, disable_bounds_checks=True,
                                             internal_scratch_in_bytes=3 * 16384),
    )(A_q, A_k, A_v, A_ssm_k, B_wqkv, B_wo,
      A_shift_k.T, A_ssm_D, gate_w,
      jnp.asarray(fwd, BF16), jnp.asarray(inv, BF16))
```
